```python
import os as _os
_os.environ.setdefault("JAX_PLATFORMS", "cpu")
import jax
import jax.numpy as jnp

def _softmax(x, axis=-1):
    return jax.nn.softmax(x, axis=axis)
def _gelu(x):
    return jax.nn.gelu(x, approximate=True)
def _silu(x):
    return jax.nn.silu(x)
def _sigmoid(x):
    return jax.nn.sigmoid(x)
def _layernorm(x, axis=-1, eps=1e-5):
    m = jnp.mean(x, axis=axis, keepdims=True)
    v = jnp.var(x, axis=axis, keepdims=True)
    return (x - m) / jnp.sqrt(v + eps)
def _scatter_add(tgt, idx, src, axis=0):
    return tgt.at[idx].add(src)
def _segment_sum(src, seg, n):
    return jax.ops.segment_sum(src, seg, n)
class _Rng:
    def __init__(self, key):
        self._k = key
    def _next(self):
        self._k, sub = jax.random.split(self._k)
        return sub
    def normal(self, shape):
        return jax.random.normal(self._next(), shape, dtype=jnp.bfloat16)
    def randint(self, lo, hi, shape):
        return jax.random.randint(self._next(), shape, lo, hi, dtype=jnp.int32)
    def uniform(self, shape, lo=0.0, hi=1.0):
        return jax.random.uniform(self._next(), shape, jnp.bfloat16, lo, hi)
    def permutation(self, n):
        return jax.random.permutation(self._next(), n)


kernel_name = 'gated_mix__compressed_kv_cla__ssm_conv_h3__prompt'

def setup_inputs():
    _rng = _Rng(jax.random.key(int.from_bytes(__import__("os").urandom(4), "little")))
    _w = (lambda a: (lambda t: t.astype(jnp.bfloat16) if jnp.issubdtype(t.dtype, jnp.floating) else t)(jnp.asarray(a)))
    def _A_setup():
        B, H, Sq, Sk, D, M = 1, 32, 2048, 2048, 128, 1024
        Dc = 4 * D
        return {
            "x": _w((lambda *s: _rng.normal(s) * 0.05)(B, Sq, M)),
            "c_kv": _w((lambda *s: _rng.normal(s) * 0.8)(B, Sk, Dc)),
            "w_q": _w((lambda *s: _rng.normal(s) * 3.2)(M, H, D) * (M ** -0.5)),
            "w_uk": _w((lambda *s: _rng.normal(s) * 3.2)(Dc, H, D) * (Dc ** -0.5)),
            "w_uv": _w((lambda *s: _rng.normal(s) * 0.8)(Dc, H, D) * (Dc ** -0.5)),
            "w_o": _w((lambda *s: _rng.normal(s) * 0.8)(H, D, M) * ((H * D) ** -0.5)),
        }
    _A_in = _A_setup()

    def _B_setup():
        B, S, D = 1, 2048, 1024
        ks = 4
        return {
            "q": _w((lambda *s: _rng.normal(s) * 0.05)(B, S, D)),
            "k": _w((lambda *s: _rng.normal(s) * 0.8)(B, S, D)),
            "v": _w((lambda *s: _rng.normal(s) * 0.8)(B, S, D)),
            "shift_k": _w((lambda *s: _rng.normal(s) * 0.8)(D, ks) * 0.5),
            "ssm_k": _w((lambda *s: _rng.normal(s) * 0.8)(D, S) * (1.0 / S ** 0.5)),
            "ssm_D": _w((lambda *s: _rng.normal(s) * 0.8)(D)),
        }
    _B_in = _B_setup()

    return {
        "A_x": _A_in["x"],
        "A_c_kv": _A_in["c_kv"],
        "A_w_q": _A_in["w_q"],
        "A_w_uk": _A_in["w_uk"],
        "A_w_uv": _A_in["w_uv"],
        "A_w_o": _A_in["w_o"],
        "B_q": _B_in["q"],
        "B_k": _B_in["k"],
        "B_v": _B_in["v"],
        "B_shift_k": _B_in["shift_k"],
        "B_ssm_k": _B_in["ssm_k"],
        "B_ssm_D": _B_in["ssm_D"],
        "gate_w": _w((lambda *s: _rng.normal(s) * 0.05)(1024) * 16.0),
    }

def reference(A_x, A_c_kv, A_w_q, A_w_uk, A_w_uv, A_w_o, B_q, B_k, B_v, B_shift_k, B_ssm_k, B_ssm_D, gate_w):
    def _A_ref(x, c_kv, w_q, w_uk, w_uv, w_o):
        B, Sq, M = x.shape[0], x.shape[1], x.shape[2]
        Sk = c_kv.shape[1]
        H, D = w_q.shape[1], w_q.shape[2]
        q = jnp.einsum("bqm,mhd->bhqd", x, w_q)
        k = jnp.einsum("bkc,chd->bhkd", c_kv, w_uk)
        v = jnp.einsum("bkc,chd->bhkd", c_kv, w_uv)
        scores = jnp.einsum("bhqd,bhkd->bhqk", q, k) * (D ** -0.5)
        off = Sk - Sq
        qi = jnp.arange(Sq)[:, None]
        kj = jnp.arange(Sk)[None, :]
        cmask = kj <= (qi + off)
        scores = jnp.where(cmask[None, None], scores, -1e9)
        p = _softmax(scores, axis=-1)
        ctx = jnp.einsum("bhqk,bhkd->bhqd", p, v)
        return jnp.einsum("bhqd,hdm->bqm", ctx, w_o)

    def _B_ref(q, k, v, shift_k, ssm_k, ssm_D):
        B, S, D = q.shape
        ks = shift_k.shape[-1]
        k_pad = jnp.pad(k, ((0, 0), (ks - 1, 0), (0, 0)))
        k_shift = jnp.zeros_like(k)
        for t in range(ks):
            k_shift = k_shift + k_pad[:, t:t + S, :] * shift_k[:, ks - 1 - t][None, None, :]
        kv = k_shift * v
        L = 2 * S
        kv_pad = jnp.pad(kv, ((0, 0), (0, S), (0, 0)))
        kf_pad = jnp.pad(ssm_k, ((0, 0), (0, S)))
        kv_f = (lambda x, axes=(-2,-1): jnp.fft.rfft2(x.astype(jnp.float32), axes=axes))(kv_pad[:, None, :, :], axes=(1, 2))
        kf_f = (lambda x, axes=(-2,-1): jnp.fft.rfft2(x.astype(jnp.float32), axes=axes))(kf_pad[:, None, :], axes=(1, 2))
        kf_f = (lambda x, *d: x.transpose(*d))(kf_f, 1, 2, 0)
        y_f = kv_f * kf_f[None, :, :, :]
        y = (lambda x, s, axes=(-2,-1): jnp.fft.irfft2(x, s=s, axes=axes).astype(jnp.bfloat16))(y_f, (1, L), axes=(1, 2))[:, 0, :S, :]
        y = y + kv * ssm_D[None, None, :]
        return q * y

    x = A_x
    g = _sigmoid((x * gate_w).sum(-1, keepdims=True))
    a = _A_ref(x, A_c_kv, A_w_q, A_w_uk, A_w_uv, A_w_o)
    b = _B_ref(x, B_k, B_v, B_shift_k, B_ssm_k, B_ssm_D)
    return g * a + (1 - g) * b
```

```python
import math

import numpy as np
import jax
import jax.numpy as jnp
import jax.experimental.pallas as pl
import jax.experimental.pallas.tpu as pltpu

CV = 3
CVS = 8
XS = 0
EQ = 4
NOBC = 0
DESC = 1

S = 2048
M = 1024
H = 32
D = 128
DC = 512
KS = 4
LANE = 128
NT_ = M // LANE
TA = 128
NA = S // TA
CB = 128
NB = S // CB
NPAIR = H // 2
WR = 2 * DC + M
WA, WB = NT_, NT_ + 1
GH = 8
NG = H // GH
NQT = 4
QR = WR // NQT
PR = 512
NXC = S // PR
NP = 16

F32 = jnp.float32
BF16 = jnp.bfloat16
NT_DIMS = (((1,), (1,)), ((), ()))
QSCALE = (D ** -0.5) * math.log2(math.e)
NEG = -1e9 * math.log2(math.e)


def _dft_mats():
    k = np.arange(CB, dtype=np.float64)[:, None]
    n = np.arange(CB, dtype=np.float64)[None, :]
    th = 2.0 * np.pi * (k + 0.5) * n / (2 * CB)
    re = np.cos(th).reshape(CB // 8, 1, 8, CB)
    im = (-np.sin(th)).reshape(CB // 8, 1, 8, CB)
    f = np.concatenate([re, im], axis=1).reshape(2 * CB, CB).astype(np.float32)
    return f, np.ascontiguousarray(f.T) / float(CB)


def _dot(a, b):
    return jnp.dot(a, b, preferred_element_type=F32)


def _dot_nt(a, b):
    return jax.lax.dot_general(a, b, NT_DIMS, preferred_element_type=F32)


def _kernel(x_hbm, c_hbm, wq_hbm, wk_hbm, wv_hbm, wo_hbm, k_hbm, v_hbm, ssm_hbm,
            shift_ref, dvec_ref, gw_ref, f_ref, finv_ref,
            out_hbm,
            x_t, c_v, lw, st,
            qa, ka, va, qb, kb, vb,
            ctx, wo_t, k_t, v_t, ssm_v, gate, kpad, out_t, wf, u_v, zref,
            sem_x, sem_c, sem_w, sem_o, sem_k, sem_v, sem_s, sem_out):

    def never(v):
        return v > jnp.inf

    def x_copy(i, r):
        rows = pl.ds(pl.multiple_of(r * PR, PR), PR)
        return pltpu.make_async_copy(x_hbm.at[rows, pl.ds(i * LANE, LANE)],
                                     x_t.at[i, rows], sem_x.at[r, i])

    def c_copy():
        return pltpu.make_async_copy(c_hbm, c_v, sem_c.at[0])

    def w_copy(g, r):
        src, r0 = ((wk_hbm, 0), (wv_hbm, 0), (wq_hbm, 0), (wq_hbm, QR))[r]
        heads = pl.ds(pl.multiple_of(g * GH, GH), GH)
        return pltpu.make_async_copy(src.at[pl.ds(r0, QR), heads, :], lw.at[pl.ds(r * QR, QR)], sem_w.at[r])

    def wo_copy(i):
        return pltpu.make_async_copy(wo_hbm.at[:, pl.ds(i * LANE, LANE)], wo_t.at[i], sem_o.at[i])

    def k_copy(i):
        return pltpu.make_async_copy(k_hbm.at[:, pl.ds(i * LANE, LANE)], k_t.at[i], sem_k.at[i])

    def v_copy(i):
        return pltpu.make_async_copy(v_hbm.at[:, pl.ds(i * LANE, LANE)], v_t.at[i], sem_v.at[i])

    def s_copy(i):
        return pltpu.make_async_copy(ssm_hbm.at[pl.ds(i * LANE, LANE), :], ssm_v.at[i], sem_s.at[i])

    def out_copy(i):
        return pltpu.make_async_copy(out_t.at[i], out_hbm.at[:, pl.ds(i * LANE, LANE)], sem_out.at[i])

    def convert(slot, r0, n, dep=None):
        w = lw[pl.ds(r0, n)].astype(F32)
        if dep is not None:
            w = jnp.where(never(dep)[None], 0.0, w)
        st[slot, pl.ds(pl.multiple_of(r0 * GH, GH), n * GH), :] = w.reshape(n * GH, D)

    def extract(h, wslot, r0, n, dep=None):
        w = st[(h // GH) % 2, pl.ds(GH * r0 + h % GH, n, stride=GH), :]
        if dep is not None:
            w = jnp.where(jnp.concatenate([never(dep)] * (n // 8), axis=0), 0.0, w)
        x_t[wslot, pl.ds(r0, n), :] = w.astype(BF16)

    def proj_kv(wslot, rows, k_out, v_out):
        wkv = jnp.concatenate([x_t[wslot, 0:DC, :], x_t[wslot, DC:2 * DC, :]], axis=1)
        kv = _dot(c_v[rows, :], wkv)
        k_out[rows, :] = kv[:, :D].astype(BF16)
        v_out[rows, :] = kv[:, D:].astype(BF16)
        return kv

    def proj_q(wslot, rows, q_out):
        xr = jnp.concatenate([x_t[i, rows, :] for i in range(NT_)], axis=1)
        q = _dot(xr, x_t[wslot, 2 * DC:WR, :])
        q_out[rows, :] = (q * QSCALE).astype(BF16)
        return q

    def gate_rows(r0, n):
        z = None
        for i in range(NT_):
            t = x_t[i, pl.ds(r0, n), :].astype(F32) * gw_ref[:, i * LANE:(i + 1) * LANE].astype(F32)
            z = t if z is None else z + t
        z = jnp.sum(z, axis=-1, keepdims=True)
        g = jnp.broadcast_to(jax.nn.sigmoid(z), (n, LANE))
        gate[pl.ds(r0, n), :] = g
        return g

    def half(h, q_ref, k_ref, v_ref, wslot, qn_ref, kn_ref, vn_ref, side_work, dep):
        row = jax.lax.broadcasted_iota(jnp.int32, (TA, TA), 0)
        col = jax.lax.broadcasted_iota(jnp.int32, (TA, TA), 1)
        tri = col <= row
        qprev = None
        for step, i in enumerate(reversed(range(NA)) if DESC else range(NA)):
            L = (i + 1) * TA
            rows = slice(i * TA, (i + 1) * TA)
            s = _dot_nt(q_ref[rows, :], k_ref[0:L, :])
            kv = proj_kv(wslot, rows, kn_ref, vn_ref)
            early_q = i >= EQ
            if early_q:
                qprev = proj_q(wslot, rows, qn_ref)[0:8]
            sd = jnp.where(tri, s[:, L - TA:], NEG)
            s = jnp.concatenate([s[:, :L - TA], sd], axis=1) if i > 0 else sd
            m = jnp.max(s, axis=-1, keepdims=True)
            mb = jnp.broadcast_to(m, (TA, LANE))
            if dep is not None:
                mb = jnp.where(dep, 0.0, mb)
            p = jnp.exp2(s - jnp.concatenate([mb] * (L // LANE), axis=1))
            l = jnp.sum(p, axis=-1, keepdims=True)
            o = _dot(p.astype(BF16), v_ref[0:L, :])
            lb = jnp.broadcast_to(l, (TA, LANE))
            r0 = pl.reciprocal(lb, approx=True)
            r1 = r0 * (2.0 - lb * r0)
            on = o * r1
            ctx[h, rows, :] = on.astype(BF16)
            pins = [qprev, qprev if early_q else sd[TA - 8:, :], kv[0:8, 0:LANE], o[0:8]]
            pin = side_work(step, pins)
            if pin is not None:
                n = pin.shape[0]
                on = jnp.concatenate([jnp.maximum(pin, on[:n]), on[n:]], axis=0)
            dep = never(on)
            if not early_q:
                qprev = proj_q(wslot, rows, qn_ref)[0:8]
        return dep

    w_copy(0, 0).start()
    w_copy(0, 1).start()
    c_copy().start()
    for c in range(NB):
        zref[c] = 0
    kpad[0:8, :] = jnp.zeros((8, LANE), F32)

    def w0_body(r, carry):
        r0 = pl.multiple_of(r * TA, TA)
        convert(0, r0, TA)
        extract(0, WA, r0, TA)
        extract(1, WB, r0, TA)
        return carry

    nq = QR // TA
    w_copy(0, 0).wait()
    jax.lax.fori_loop(0, nq, w0_body, 0)
    w_copy(0, 1).wait()
    if XS == 0:
        w_copy(0, 2).start()
        w_copy(0, 3).start()
    jax.lax.fori_loop(nq, 2 * nq, w0_body, 0)
    c_copy().wait()
    if XS == 1:
        w_copy(0, 2).start()
        w_copy(0, 3).start()

    def kv0_body(r, carry):
        for i in range(NT_):
            x_copy(i, r).start()
        proj_kv(WA, pl.ds(pl.multiple_of(r * PR, PR), PR), ka, va)
        return carry

    jax.lax.fori_loop(0, S // PR, kv0_body, 0)
    w_copy(0, 2).wait()
    w_copy(0, 3).wait()
    jax.lax.fori_loop(2 * nq, 4 * nq, w0_body, 0)

    def q0_body(r, carry):
        for i in range(NT_):
            x_copy(i, r).wait()
        proj_q(WA, pl.ds(pl.multiple_of(r * PR, PR), PR), qa)
        return carry

    jax.lax.fori_loop(0, NXC, q0_body, 0)
    for r in range(NQT):
        w_copy(1, r).start()

    def pair_body(j, carry):
        for r in range(NQT):
            @pl.when(jnp.logical_and(j < (NG - 1) * NQT, j % NQT == r))
            def _():
                w_copy(j // NQT + 1, r).wait()

            @pl.when(jnp.logical_and(jnp.logical_and(j >= 1, j <= (NG - 2) * NQT), (j - 1) % NQT == r))
            def _():
                w_copy((j - 1) // NQT + 2, r).start()

        @pl.when(jnp.logical_and(j >= 1, j <= NT_))
        def _():
            k_copy(j - 1).start()
            v_copy(j - 1).start()
            s_copy(j - 1).start()
            wo_copy(j - 1).start()

        z = zref[0]
        gslot = jnp.minimum(j // NQT + 1, NG - 1) % 2
        q0 = pl.multiple_of((j % NQT) * QR, QR)
        hn = jnp.minimum(2 * j + 2, H - 2)

        def side1(step, pins):
            extract(hn, z + WA, step * TA, TA, pins[1])
            if step < CVS:
                n = QR // CVS // 2
                for t in range(2):
                    convert(gslot, q0 + (step * 2 + t) * n, n, pins[2 + t])
            return None

        def side2(step, pins):
            extract(hn + 1, z + WB, step * TA, TA, pins[1])
            return gate_rows(pl.multiple_of(j * TA + step * 8, 8), 8)

        dep = half(2 * j, qa, ka, va, WB, qb, kb, vb, side1, None)
        half(2 * j + 1, qb, kb, vb, WA, qa, ka, va, side2, dep)
        return carry

    jax.lax.fori_loop(0, NPAIR, pair_body, 0)

    sgn_row = jax.lax.broadcasted_iota(jnp.int32, (8, LANE), 0)
    sgn = jnp.where((sgn_row & 1) == 0, 1.0, -1.0).astype(F32)

    def conv_fwd(i):
        fwd = f_ref[...]
        sh = shift_ref[i].astype(F32)
        kpad[8:8 + S, :] = k_t[i].astype(F32)
        hprev = None
        for b in range(NB):
            ks = None
            for t in range(KS):
                term = kpad[8 + b * CB - t:8 + (b + 1) * CB - t, :] * sh[t:t + 1, :]
                ks = term if ks is None else ks + term
            u = (ks * v_t[i, b * CB:(b + 1) * CB, :].astype(F32)).astype(BF16)
            u_v[b * CB:(b + 1) * CB, :] = u
            ufb = _dot(fwd, u)
            hf = _dot_nt(fwd, ssm_v[i, :, b * CB:(b + 1) * CB])
            for sl in range(CB // 8):
                re = slice(16 * sl, 16 * sl + 8)
                im = slice(16 * sl + 8, 16 * sl + 16)
                wf[b, 32 * sl:32 * sl + 16, :] = ufb[16 * sl:16 * sl + 16]
                if hprev is None:
                    wf[b, 32 * sl + 16:32 * sl + 32, :] = hf[16 * sl:16 * sl + 16]
                else:
                    wf[b, 32 * sl + 16:32 * sl + 24, :] = hf[re] - sgn * hprev[im]
                    wf[b, 32 * sl + 24:32 * sl + 32, :] = hf[im] + sgn * hprev[re]
            hprev = hf

    def tile_waits(i):
        k_copy(i).wait()
        v_copy(i).wait()
        s_copy(i).wait()

    tile_waits(0)
    conv_fwd(0)

    def tile_body(i, carry):
        wo_copy(i).wait()

        @pl.when(i + 1 < NT_)
        def _():
            tile_waits(i + 1)

        dv = dvec_ref[i].astype(F32)
        hp = H // NP
        for cblk in range(NB):
            rows = slice(cblk * CB, (cblk + 1) * CB)
            z = zref[cblk]
            a = None
            for kp in range(NP):
                for sl in range(kp * (16 // NP), (kp + 1) * (16 // NP)):
                    yr = None
                    yi = None
                    for b in range(cblk + 1):
                        a_r = wf[z + b, pl.ds(32 * sl, 8), :]
                        a_i = wf[z + b, pl.ds(32 * sl + 8, 8), :]
                        g_r = wf[z + (cblk - b), pl.ds(32 * sl + 16, 8), :]
                        g_i = wf[z + (cblk - b), pl.ds(32 * sl + 24, 8), :]
                        tr = a_r * g_r - a_i * g_i
                        ti = a_r * g_i + a_i * g_r
                        yr = tr if yr is None else yr + tr
                        yi = ti if yi is None else yi + ti
                    ctx[z + H, 16 * sl:16 * sl + 16, :] = jnp.concatenate([yr, yi], axis=0).astype(BF16)
                cr = jnp.concatenate([ctx[h, rows, :] for h in range(kp * hp, (kp + 1) * hp)], axis=1)
                ap = _dot(cr, wo_t[i, kp * hp * D:(kp + 1) * hp * D, :])
                a = ap if a is None else a + ap
            y = _dot(finv_ref[...], ctx[H, 0:2 * CB, :]) + u_v[rows, :].astype(F32) * dv
            bb = x_t[i, rows, :].astype(F32) * y
            g = gate[rows, :]
            out_t[i, rows, :] = (g * a + (1.0 - g) * bb).astype(BF16)
        out_copy(i).start()
        conv_fwd(jnp.minimum(i + 1, NT_ - 1))
        return carry

    jax.lax.fori_loop(0, NT_, tile_body, 0)
    for i in range(NT_):
        out_copy(i).wait()


@jax.jit
def pallas_gated_mix__compressed_kv_cla__ssm_conv_h3__prompt_kernel(
    A_x: jax.Array,
    A_c_kv: jax.Array,
    A_w_q: jax.Array,
    A_w_uk: jax.Array,
    A_w_uv: jax.Array,
    A_w_o: jax.Array,
    B_q: jax.Array,
    B_k: jax.Array,
    B_v: jax.Array,
    B_shift_k: jax.Array,
    B_ssm_k: jax.Array,
    B_ssm_D: jax.Array,
    gate_w: jax.Array,
):
    del B_q
    fwd, finv = _dft_mats()
    x = A_x.reshape(S, M)
    c = A_c_kv.reshape(S, DC)
    wo = A_w_o.reshape(H * D, M)
    kk = B_k.reshape(S, M)
    vv = B_v.reshape(S, M)
    shift = B_shift_k.reshape(NT_, LANE, KS).transpose(0, 2, 1)
    dvec = B_ssm_D.reshape(NT_, 1, LANE)
    gw = gate_w.reshape(1, M)

    any_spec = pl.BlockSpec(memory_space=pl.ANY)
    vmem_spec = pl.BlockSpec(memory_space=pltpu.VMEM)
    out = pl.pallas_call(
        _kernel,
        out_shape=jax.ShapeDtypeStruct((S, M), BF16),
        in_specs=[any_spec] * 9 + [vmem_spec] * 5,
        out_specs=any_spec,
        scratch_shapes=[
            pltpu.VMEM((NT_ + 2, S, LANE), BF16),
            pltpu.VMEM((S, DC), BF16),
            pltpu.VMEM((WR, GH, D), BF16),
            pltpu.VMEM((2, WR * GH, D), F32),
            pltpu.VMEM((S, D), BF16),
            pltpu.VMEM((S, D), BF16),
            pltpu.VMEM((S, D), BF16),
            pltpu.VMEM((S, D), BF16),
            pltpu.VMEM((S, D), BF16),
            pltpu.VMEM((S, D), BF16),
            pltpu.VMEM((H + 1, S, D), BF16),
            pltpu.VMEM((NT_, H * D, LANE), BF16),
            pltpu.VMEM((NT_, S, LANE), BF16),
            pltpu.VMEM((NT_, S, LANE), BF16),
            pltpu.VMEM((NT_, LANE, S), BF16),
            pltpu.VMEM((S, LANE), F32),
            pltpu.VMEM((S + 8, LANE), F32),
            pltpu.VMEM((NT_, S, LANE), BF16),
            pltpu.VMEM((NB, 4 * CB, LANE), F32),
            pltpu.VMEM((S, LANE), BF16),
            pltpu.SMEM((NB,), jnp.int32),
            pltpu.SemaphoreType.DMA((NXC, NT_)),
            pltpu.SemaphoreType.DMA((1,)),
            pltpu.SemaphoreType.DMA((NQT,)),
            pltpu.SemaphoreType.DMA((NT_,)),
            pltpu.SemaphoreType.DMA((NT_,)),
            pltpu.SemaphoreType.DMA((NT_,)),
            pltpu.SemaphoreType.DMA((NT_,)),
            pltpu.SemaphoreType.DMA((NT_,)),
        ],
        compiler_params=pltpu.CompilerParams(vmem_limit_bytes=120 * 1024 * 1024,
                                             disable_bounds_checks=bool(NOBC)),
    )(x, c, A_w_q, A_w_uk, A_w_uv, wo, kk, vv, B_ssm_k,
      shift, dvec, gw, jnp.asarray(fwd, BF16), jnp.asarray(finv, BF16))
    return out.reshape(1, S, M)
```

```python
import math

import numpy as np
import jax
import jax.numpy as jnp
import jax.experimental.pallas as pl
import jax.experimental.pallas.tpu as pltpu

CV = 3
CVS = 8
XS = 0
EQ = 1
MIDW = 0
CV0 = 0
PLAG = 4
NOHEAD = 0
NOTAIL = 0
HEXT = 0
INVP = 2
FP0 = 4
FP1 = 4
NOBC = 0
DESC = 1

S = 2048
M = 1024
H = 32
D = 128
DC = 512
KS = 4
LANE = 128
NT_ = M // LANE
TA = 128
NA = S // TA
CB = 128
NB = S // CB
NPAIR = H // 2
WR = 2 * DC + M
WA, WB = NT_, NT_ + 1
GH = 8
NG = H // GH
NQT = 4
QR = WR // NQT
PR = 512
NXC = S // PR
NP = 8

F32 = jnp.float32
BF16 = jnp.bfloat16
NT_DIMS = (((1,), (1,)), ((), ()))
QSCALE = (D ** -0.5) * math.log2(math.e)
NEG = -1e9 * math.log2(math.e)


def _dft_mats():
    k = np.arange(CB, dtype=np.float64)[:, None]
    n = np.arange(CB, dtype=np.float64)[None, :]
    th = 2.0 * np.pi * (k + 0.5) * n / (2 * CB)
    re = np.cos(th).reshape(CB // 8, 1, 8, CB)
    im = (-np.sin(th)).reshape(CB // 8, 1, 8, CB)
    f = np.concatenate([re, im], axis=1).reshape(2 * CB, CB).astype(np.float32)
    return f, np.ascontiguousarray(f.T) / float(CB)


def _dot(a, b):
    return jnp.dot(a, b, preferred_element_type=F32)


def _dot_nt(a, b):
    return jax.lax.dot_general(a, b, NT_DIMS, preferred_element_type=F32)


def _kernel(x_hbm, c_hbm, wq_hbm, wk_hbm, wv_hbm, wo_hbm, k_hbm, v_hbm, ssm_hbm,
            shift_ref, dvec_ref, gw_ref, f_ref, finv_ref,
            out_hbm,
            x_t, c_v, lw, st,
            qa, ka, va, kb, vb,
            ctx, wo_t, k_t, v_t, ssm_v, gate, kpad, out_t, u_v, bpart, zref,
            sem_x, sem_c, sem_w, sem_t, sem_out, *wf):

    def never(v):
        return v > jnp.inf

    def x_copy(i, r):
        rows = pl.ds(pl.multiple_of(r * PR, PR), PR)
        return pltpu.make_async_copy(x_hbm.at[rows, pl.ds(i * LANE, LANE)],
                                     x_t.at[i, rows], sem_x.at[0])

    def c_copy():
        return pltpu.make_async_copy(c_hbm, c_v, sem_c.at[0])

    def w_copy(g, r):
        src, r0 = ((wk_hbm, 0), (wv_hbm, 0), (wq_hbm, 0), (wq_hbm, QR))[r]
        heads = pl.ds(pl.multiple_of(g * GH, GH), GH)
        return pltpu.make_async_copy(src.at[pl.ds(r0, QR), heads, :], lw.at[pl.ds(r * QR, QR)], sem_w.at[r])

    def tile_copies(i):
        cols = pl.ds(i * LANE, LANE)
        return [
            pltpu.make_async_copy(k_hbm.at[:, cols], k_t.at[i], sem_t.at[i]),
            pltpu.make_async_copy(v_hbm.at[:, cols], v_t.at[i], sem_t.at[i]),
            pltpu.make_async_copy(ssm_hbm.at[cols, :], ssm_v.at[i], sem_t.at[i]),
            pltpu.make_async_copy(wo_hbm.at[:, cols], wo_t.at[i], sem_t.at[i]),
        ]

    def out_copy(i):
        return pltpu.make_async_copy(out_t.at[i], out_hbm.at[:, pl.ds(i * LANE, LANE)], sem_out.at[0])

    def convert(slot, r0, n, dep=None):
        w = lw[pl.ds(r0, n)].astype(F32)
        if dep is not None:
            w = jnp.where(never(dep)[None], 0.0, w)
        st[slot, pl.ds(pl.multiple_of(r0 * GH, GH), n * GH), :] = w.reshape(n * GH, D)

    def extract(h, wslot, r0, n, dep=None):
        w = st[(h // GH) % 2, pl.ds(GH * r0 + h % GH, n, stride=GH), :]
        if dep is not None:
            w = jnp.where(jnp.concatenate([never(dep)] * (n // 8), axis=0), 0.0, w)
        x_t[wslot, pl.ds(r0, n), :] = w.astype(BF16)

    def proj_kv(wslot, rows, k_out, v_out):
        wkv = jnp.concatenate([x_t[wslot, 0:DC, :], x_t[wslot, DC:2 * DC, :]], axis=1)
        kv = _dot(c_v[rows, :], wkv)
        k_out[rows, :] = kv[:, :D].astype(BF16)
        v_out[rows, :] = kv[:, D:].astype(BF16)
        return kv

    def proj_q(wslot, rows):
        xr = jnp.concatenate([x_t[i, rows, :] for i in range(NT_)], axis=1)
        return _dot(xr, x_t[wslot, 2 * DC:WR, :]) * QSCALE

    def gate_rows(r0, n):
        z = None
        for i in range(NT_):
            t = x_t[i, pl.ds(r0, n), :].astype(F32) * gw_ref[:, i * LANE:(i + 1) * LANE].astype(F32)
            z = t if z is None else z + t
        z = jnp.sum(z, axis=-1, keepdims=True)
        g = jnp.broadcast_to(jax.nn.sigmoid(z), (n, LANE))
        gate[pl.ds(r0, n), :] = g
        return g

    def blk(i):
        return slice(i * TA, (i + 1) * TA)

    def half(h, k_ref, v_ref, wcur, wnext, kn_ref, vn_ref, q, side_work, dep):
        row = jax.lax.broadcasted_iota(jnp.int32, (TA, TA), 0)
        col = jax.lax.broadcasted_iota(jnp.int32, (TA, TA), 1)
        tri = col <= row
        for step, i in enumerate(reversed(range(NA))):
            L = (i + 1) * TA
            s = _dot_nt(q, k_ref[0:L, :])
            qn = proj_q(wcur, blk(i - 1)) if i > 0 else proj_q(wnext, blk(NA - 1))
            q = qn.astype(BF16)
            early = i >= EQ
            if early:
                kv = proj_kv(wnext, blk(step), kn_ref, vn_ref)
            sd = jnp.where(tri, s[:, L - TA:], NEG)
            s = jnp.concatenate([s[:, :L - TA], sd], axis=1) if i > 0 else sd
            m = jnp.max(s, axis=-1, keepdims=True)
            mb = jnp.broadcast_to(m, (TA, LANE))
            if dep is not None:
                mb = jnp.where(dep, 0.0, mb)
            p = jnp.exp2(s - jnp.concatenate([mb] * (L // LANE), axis=1))
            l = jnp.sum(p, axis=-1, keepdims=True)
            o = _dot(p.astype(BF16), v_ref[0:L, :])
            lb = jnp.broadcast_to(l, (TA, LANE))
            r0 = pl.reciprocal(lb, approx=True)
            r1 = r0 * (2.0 - lb * r0)
            on = o * r1
            ctx[h, blk(i), :] = on.astype(BF16)
            pins = [kv[0:8, 0:LANE] if early else qn[0:8], qn[0:8], o[0:8]]
            pin = side_work(step, pins)
            if pin is not None:
                n = pin.shape[0]
                on = jnp.concatenate([jnp.maximum(pin, on[:n]), on[n:]], axis=0)
            dep = never(on)
            if not early:
                proj_kv(wnext, blk(step), kn_ref, vn_ref)
        return q, dep

    w_copy(0, 0).start()
    w_copy(0, 1).start()
    c_copy().start()
    for c in range(NB):
        zref[c] = 0
    kpad[0:8, :] = jnp.zeros((8, LANE), F32)

    def w0_body(r, carry):
        r0 = pl.multiple_of(r * TA, TA)
        convert(0, r0, TA)
        extract(0, WA, r0, TA)
        extract(1, WB, r0, TA)
        return carry

    nq = QR // TA
    w_copy(0, 0).wait()
    jax.lax.fori_loop(0, nq, w0_body, 0)
    w_copy(0, 1).wait()
    w_copy(0, 2).start()
    w_copy(0, 3).start()
    jax.lax.fori_loop(nq, 2 * nq, w0_body, 0)
    c_copy().wait()

    def kv0_body(r, carry):
        for i in range(NT_):
            x_copy(i, NXC - 1 - r).start()
        proj_kv(WA, pl.ds(pl.multiple_of(r * PR, PR), PR), ka, va)
        return carry

    jax.lax.fori_loop(0, S // PR, kv0_body, 0)
    w_copy(0, 2).wait()
    w_copy(0, 3).wait()
    jax.lax.fori_loop(2 * nq, 4 * nq, w0_body, 0)
    for r in range(NQT):
        w_copy(1, r).start()
    for r in range(NXC):
        for i in range(NT_):
            x_copy(i, r).wait()
    qa[...] = proj_q(WA, blk(NA - 1)).astype(BF16)

    def pair_body(j, carry):
        for r in range(NQT):
            @pl.when(jnp.logical_and(j < (NG - 1) * NQT, j % NQT == r))
            def _():
                w_copy(j // NQT + 1, r).wait()

        for t in range(1, NT_ + 1):
            @pl.when(j == t)
            def _():
                w_copy((t - 1) // NQT + 2, (t - 1) % NQT).start()
                for cp in tile_copies(t - 1):
                    cp.start()

        z = zref[0]
        gslot = jnp.minimum(j // NQT + 1, NG - 1) % 2
        q0 = pl.multiple_of((j % NQT) * QR, QR)
        hn = jnp.minimum(2 * j + 2, H - 2)
        nh = NA // 2

        def extract_step(step, hq, wq_slot, hkv, wkv_slot, pin):
            chunks = [2 * step, 2 * step + 1] if step < EQ else ([step + EQ] if step + EQ < NA else [])
            for ch in chunks:
                if ch < nh:
                    extract(hq, z + wq_slot, 2 * DC + ch * TA, TA, pin)
                else:
                    extract(hkv, z + wkv_slot, (ch - nh) * TA, TA, pin)

        def side1(step, pins):
            extract_step(step, 2 * j + 1, WB, hn, WA, pins[0])
            if CV0 <= step < CV0 + CVS:
                n = QR // CVS // 2
                for t in range(2):
                    convert(gslot, q0 + ((step - CV0) * 2 + t) * n, n, pins[1 + t])
            return None

        def side2(step, pins):
            extract_step(step, hn, WA, hn + 1, WB, pins[0])
            return gate_rows(pl.multiple_of(j * TA + step * 8, 8), 8)

        q, dep = half(2 * j, ka, va, WA, WB, kb, vb, qa[...], side1, None)
        q, _ = half(2 * j + 1, kb, vb, WB, WA, ka, va, q, side2, dep)
        qa[...] = q
        return carry

    if not NOHEAD:
        jax.lax.fori_loop(0, NPAIR, pair_body, 0)

    sgn_row = jax.lax.broadcasted_iota(jnp.int32, (8, LANE), 0)
    sgn = jnp.where((sgn_row & 1) == 0, 1.0, -1.0).astype(F32)

    for i in range(NT_):
        for cp in tile_copies(i):
            cp.wait()

    RB = 2 * CB
    NR = S // RB
    hp = H // NP
    npin = 32 // NP
    rg = RB // npin

    def tile_body(i, carry):
        sh = shift_ref[i].astype(F32)
        dv = dvec_ref[i].astype(F32)
        hprev = [None]
        hist = []

        def fwd(b):
            hf = _dot_nt(f_ref[...], ssm_v[i, :, b * CB:(b + 1) * CB])
            kpad[8 + b * CB:8 + (b + 1) * CB, :] = k_t[i, b * CB:(b + 1) * CB, :].astype(F32)
            ks = None
            for t in range(KS):
                term = kpad[8 + b * CB - t:8 + (b + 1) * CB - t, :] * sh[t:t + 1, :]
                ks = term if ks is None else ks + term
            u = (ks * v_t[i, b * CB:(b + 1) * CB, :].astype(F32)).astype(BF16)
            u_v[b * CB:(b + 1) * CB, :] = u
            ufb = _dot(f_ref[...], u)
            w = wf[b // 2]
            for sl in range(CB // 8):
                re = slice(16 * sl, 16 * sl + 8)
                im = slice(16 * sl + 8, 16 * sl + 16)
                w[b % 2, 32 * sl:32 * sl + 16, :] = ufb[16 * sl:16 * sl + 16]
                if hprev[0] is None:
                    w[b % 2, 32 * sl + 16:32 * sl + 32, :] = hf[16 * sl:16 * sl + 16]
                else:
                    w[b % 2, 32 * sl + 16:32 * sl + 24, :] = hf[re] - sgn * hprev[0][im]
                    w[b % 2, 32 * sl + 24:32 * sl + 32, :] = hf[im] + sgn * hprev[0][re]
            hprev[0] = hf
            if HEXT & 1:
                hist.extend([hf[0:8], ufb[0:8]])

        def mac(cblk, sl, pin):
            z = zref[cblk]
            yr = None
            yi = None
            for b in range(cblk + 1):
                wu, wg = wf[b // 2], wf[(cblk - b) // 2]
                a_r = wu[z + b % 2, pl.ds(32 * sl, 8), :]
                a_i = wu[z + b % 2, pl.ds(32 * sl + 8, 8), :]
                g_r = wg[z + (cblk - b) % 2, pl.ds(32 * sl + 16, 8), :]
                g_i = wg[z + (cblk - b) % 2, pl.ds(32 * sl + 24, 8), :]
                tr = a_r * g_r - a_i * g_i
                ti = a_r * g_i + a_i * g_r
                yr = tr if yr is None else yr + tr
                yi = ti if yi is None else yi + ti
            if pin is not None:
                yr = jnp.where(never(pin), 0.0, yr)
            y0 = (cblk % 8) * 2 * CB + 16 * sl
            ctx[z + H, y0:y0 + 16, :] = jnp.concatenate([yr, yi], axis=0).astype(BF16)

        def inv(r):
            y = jnp.concatenate(
                [_dot(finv_ref[...], ctx[H, (c % 8) * 2 * CB:(c % 8 + 1) * 2 * CB, :]) for c in (2 * r, 2 * r + 1)],
                axis=0)
            if HEXT & 2:
                hist.extend([y[0:8], y[CB:CB + 8]])
            rows = slice(r * RB, (r + 1) * RB)
            y = y + u_v[rows, :].astype(F32) * dv
            bpart[r % 2] = (1.0 - gate[rows, :]) * (x_t[i, rows, :].astype(F32) * y)

        for b in range(4):
            fwd(b)
        for r in range(NR):
            cones = [(2 * (r + 1) + k % 2, k // 2) for k in range(32)] if r + 1 < NR else []
            if r == 0:
                cones = [(k % 2, k // 2) for k in range(32)] + cones
            first = npin if r == 0 else 0
            npts = NP * npin - first
            a = None
            for kp in range(NP):
                parts = []
                for t in range(npin):
                    pt = kp * npin + t - first
                    if pt >= 0:
                        for cn in cones[pt * len(cones) // npts:(pt + 1) * len(cones) // npts]:
                            hi = len(hist) + t - PLAG
                            mac(*cn, hist[hi] if hi >= 0 else None)
                    rows = slice(r * RB + t * rg, r * RB + (t + 1) * rg)
                    parts.append(jnp.concatenate([ctx[h, rows, :] for h in range(kp * hp, (kp + 1) * hp)], axis=1))
                ap = _dot(jnp.concatenate(parts, axis=0), wo_t[i, kp * hp * D:(kp + 1) * hp * D, :])
                a = ap if a is None else ap + a
                hist.extend([a[t * rg:t * rg + 8] for t in range(npin)])
                if (kp == INVP and r > 0) or (kp == NP - 2 and r == 0):
                    inv(r)
                for e, fp in enumerate((FP0, FP1)):
                    if kp == fp and 2 * r + 4 + e < NB:
                        fwd(2 * r + 4 + e)
            rows = slice(r * RB, (r + 1) * RB)
            out_t[i, rows, :] = (gate[rows, :] * a + bpart[r % 2]).astype(BF16)
        out_copy(i).start()
        return carry

    if not NOTAIL:
        jax.lax.fori_loop(0, NT_, tile_body, 0)
    for i in range(NT_):
        out_copy(i).wait()


@jax.jit
def pallas_gated_mix__compressed_kv_cla__ssm_conv_h3__prompt_kernel(
    A_x: jax.Array,
    A_c_kv: jax.Array,
    A_w_q: jax.Array,
    A_w_uk: jax.Array,
    A_w_uv: jax.Array,
    A_w_o: jax.Array,
    B_q: jax.Array,
    B_k: jax.Array,
    B_v: jax.Array,
    B_shift_k: jax.Array,
    B_ssm_k: jax.Array,
    B_ssm_D: jax.Array,
    gate_w: jax.Array,
):
    del B_q
    fwd, finv = _dft_mats()
    x = A_x.reshape(S, M)
    c = A_c_kv.reshape(S, DC)
    wo = A_w_o.reshape(H * D, M)
    kk = B_k.reshape(S, M)
    vv = B_v.reshape(S, M)
    shift = B_shift_k.reshape(NT_, LANE, KS).transpose(0, 2, 1)
    dvec = B_ssm_D.reshape(NT_, 1, LANE)
    gw = gate_w.reshape(1, M)

    any_spec = pl.BlockSpec(memory_space=pl.ANY)
    vmem_spec = pl.BlockSpec(memory_space=pltpu.VMEM)
    out = pl.pallas_call(
        _kernel,
        out_shape=jax.ShapeDtypeStruct((S, M), BF16),
        in_specs=[any_spec] * 9 + [vmem_spec] * 5,
        out_specs=any_spec,
        scratch_shapes=[
            pltpu.VMEM((NT_ + 2, S, LANE), BF16),
            pltpu.VMEM((S, DC), BF16),
            pltpu.VMEM((WR, GH, D), BF16),
            pltpu.VMEM((2, WR * GH, D), F32),
            pltpu.VMEM((TA, D), BF16),
            pltpu.VMEM((S, D), BF16),
            pltpu.VMEM((S, D), BF16),
            pltpu.VMEM((S, D), BF16),
            pltpu.VMEM((S, D), BF16),
            pltpu.VMEM((H + 1, S, D), BF16),
            pltpu.VMEM((NT_, H * D, LANE), BF16),
            pltpu.VMEM((NT_, S, LANE), BF16),
            pltpu.VMEM((NT_, S, LANE), BF16),
            pltpu.VMEM((NT_, LANE, S), BF16),
            pltpu.VMEM((S, LANE), F32),
            pltpu.VMEM((S + 32, LANE), F32),
            pltpu.VMEM((NT_, S, LANE), BF16),
            pltpu.VMEM((S, LANE), BF16),
            pltpu.VMEM((2, 2 * CB, LANE), F32),
            pltpu.SMEM((NB,), jnp.int32),
            pltpu.SemaphoreType.DMA((1,)),
            pltpu.SemaphoreType.DMA((1,)),
            pltpu.SemaphoreType.DMA((NQT,)),
            pltpu.SemaphoreType.DMA((NT_,)),
            pltpu.SemaphoreType.DMA((1,)),
        ] + [pltpu.VMEM((2, 4 * CB, LANE), F32)] * (NB // 2),
        compiler_params=pltpu.CompilerParams(vmem_limit_bytes=120 * 1024 * 1024,
                                             disable_bounds_checks=bool(NOBC)),
    )(x, c, A_w_q, A_w_uk, A_w_uv, wo, kk, vv, B_ssm_k,
      shift, dvec, gw, jnp.asarray(fwd, BF16), jnp.asarray(finv, BF16))
    return out.reshape(1, S, M)
```

```python
import math

import numpy as np
import jax
import jax.numpy as jnp
import jax.experimental.pallas as pl
import jax.experimental.pallas.tpu as pltpu

CV = 3
CVS = 8
XS = 0
EQ = 1
MIDW = 0
CV0 = 0
PLAG = 4
NOHEAD = 0
NOTAIL = 0
HEXT = 0
INVP = 2
FP0 = 4
FP1 = 4
OL = 512
AH = 4
NW = 8
CG0 = 4
QFIRST = 1
Q0 = 0
ND = 3
LA = 16
LQ2 = 1
LQ0 = 1
XT0 = 2
NOBC = 0
DESC = 1

S = 2048
M = 1024
H = 32
D = 128
DC = 512
KS = 4
LANE = 128
NT_ = M // LANE
TA = 128
NA = S // TA
CB = 128
NB = S // CB
NPAIR = H // 2
WR = 2 * DC + M
WA, WB = NT_, NT_ + 1
GH = 8
NG = H // GH
NQT = 4
QR = WR // NQT
PR = 512
NCC = S // PR
NP = 8

F32 = jnp.float32
BF16 = jnp.bfloat16
NT_DIMS = (((1,), (1,)), ((), ()))
QSCALE = (D ** -0.5) * math.log2(math.e)
NEG = -1e9 * math.log2(math.e)


def _dft_mats():
    k = np.arange(CB, dtype=np.float64)[:, None]
    n = np.arange(CB, dtype=np.float64)[None, :]
    th = 2.0 * np.pi * (k + 0.5) * n / (2 * CB)
    re = np.cos(th).reshape(CB // 8, 1, 8, CB)
    im = (-np.sin(th)).reshape(CB // 8, 1, 8, CB)
    f = np.concatenate([re, im], axis=1).reshape(2 * CB, CB).astype(np.float32)
    return f, np.ascontiguousarray(f.T) / float(CB)


def _dot(a, b):
    return jnp.dot(a, b, preferred_element_type=F32)


def _dot_nt(a, b):
    return jax.lax.dot_general(a, b, NT_DIMS, preferred_element_type=F32)


def _kernel(x_hbm, c_hbm, wq_hbm, wk_hbm, wv_hbm, wo_hbm, k_hbm, v_hbm, ssm_hbm,
            shift_hbm, dvec_hbm, gw_hbm, f_hbm, finv_hbm,
            out_hbm,
            x_t, c_v, lw, st,
            qa, kbuf, vbuf,
            ctx, wo_t, k_t, v_t, ssm_v, gate, kpad, out_t, u_v, bpart,
            wf0, wf1, wf2, wf3, wf4, wf5, wf6, wf7,
            f_ref, finv_ref, dtile, shift_ref, dvec_ref, gw_ref, zref,
            sem_x, sem_c, sem_w, sem_t, sem_out, sem_s):

    wf = (wf0, wf1, wf2, wf3, wf4, wf5, wf6, wf7)

    def never(v):
        return v > jnp.inf

    def x_copy(i):
        return pltpu.make_async_copy(x_hbm.at[:, pl.ds(i * LANE, LANE)], x_t.at[i], sem_x.at[0])

    def c_copy(r):
        rows = pl.ds(pl.multiple_of(r * PR, PR), PR)
        return pltpu.make_async_copy(c_hbm.at[rows], c_v.at[rows], sem_c.at[r])

    def w_copy(g, r):
        src, r0 = ((wk_hbm, 0), (wv_hbm, 0), (wq_hbm, 0), (wq_hbm, QR))[r]
        heads = pl.ds(pl.multiple_of(g * GH, GH), GH)
        return pltpu.make_async_copy(src.at[pl.ds(r0, QR), heads, :], lw.at[pl.ds(r * QR, QR)], sem_w.at[r])

    def tile_copies(i):
        cols = pl.ds(i * LANE, LANE)
        return [
            pltpu.make_async_copy(k_hbm.at[:, cols], k_t.at[i], sem_t.at[i]),
            pltpu.make_async_copy(v_hbm.at[:, cols], v_t.at[i], sem_t.at[i]),
            pltpu.make_async_copy(ssm_hbm.at[cols, :], ssm_v.at[i], sem_t.at[i]),
            pltpu.make_async_copy(wo_hbm.at[:, cols], wo_t.at[i], sem_t.at[i]),
        ]

    def out_copy(i, part):
        rows = (pl.ds(0, S - OL), pl.ds(S - OL, OL))[part]
        return pltpu.make_async_copy(out_t.at[i, rows], out_hbm.at[rows, pl.ds(i * LANE, LANE)], sem_out.at[0])

    def small_copies():
        return [pltpu.make_async_copy(src, dst, sem_s.at[0])
                for src, dst in ((shift_hbm, shift_ref), (dvec_hbm, dvec_ref), (gw_hbm, gw_ref),
                                 (f_hbm, f_ref), (finv_hbm, finv_ref))]

    def convert(slot, r0, n, dep=None):
        w = lw[pl.ds(r0, n)].astype(F32)
        if dep is not None:
            w = jnp.where(never(dep)[None], 0.0, w)
        st[slot, pl.ds(pl.multiple_of(r0 * GH, GH), n * GH), :] = w.reshape(n * GH, D)

    def extract(h, wslot, r0, n, dep=None):
        w = st[(h // GH) % 2, pl.ds(GH * r0 + h % GH, n, stride=GH), :]
        if dep is not None:
            w = jnp.where(jnp.concatenate([never(dep)] * (n // 8), axis=0), 0.0, w)
        x_t[wslot, pl.ds(r0, n), :] = w.astype(BF16)

    def wslot_of(h):
        return NT_ + h % NW

    def proj_q(wslot, rows):
        xr = jnp.concatenate([x_t[i, rows, :] for i in range(NT_)], axis=1)
        return _dot(xr, x_t[wslot, 2 * DC:WR, :]) * QSCALE

    def gate_rows(r0, n):
        gw = gw_ref[...].astype(F32)
        z = None
        for i in range(NT_):
            t = x_t[i, pl.ds(r0, n), :].astype(F32) * gw[i:i + 1, :]
            z = t if z is None else z + t
        z = jnp.sum(z, axis=-1, keepdims=True)
        g = jnp.broadcast_to(jax.nn.sigmoid(z), (n, LANE))
        gate[pl.ds(r0, n), :] = g
        return g

    def blk(i):
        return slice(i * TA, (i + 1) * TA)

    def softmax_pv(h, slot, i, s, dep):
        L = (i + 1) * TA
        row = jax.lax.broadcasted_iota(jnp.int32, (TA, TA), 0)
        col = jax.lax.broadcasted_iota(jnp.int32, (TA, TA), 1)
        sd = jnp.where(col <= row, s[:, L - TA:], NEG)
        s = jnp.concatenate([s[:, :L - TA], sd], axis=1) if i > 0 else sd
        m = jnp.max(s, axis=-1, keepdims=True)
        mb = jnp.broadcast_to(m, (TA, LANE))
        if dep is not None:
            mb = jnp.where(dep, 0.0, mb)
        p = jnp.exp2(s - jnp.concatenate([mb] * (L // LANE), axis=1))
        l = jnp.sum(p, axis=-1, keepdims=True)
        o = _dot(p.astype(BF16), vbuf[slot, 0:L, :])
        lb = jnp.broadcast_to(l, (TA, LANE))
        r0 = pl.reciprocal(lb, approx=True)
        r1 = r0 * (2.0 - lb * r0)
        on = o * r1
        ctx[h, blk(i), :] = on.astype(BF16)
        return o, on

    def head_full(h, side_work):
        slot = h % AH
        wcur, wnext, wkv_slot = wslot_of(h), wslot_of(h + 1), wslot_of(h + AH)

        def pkv(c):
            wkv = jnp.concatenate([x_t[wkv_slot, 0:DC, :], x_t[wkv_slot, DC:2 * DC, :]], axis=1)
            kv = _dot(c_v[blk(c), :], wkv)
            kbuf[slot, blk(c), :] = kv[:, :D].astype(BF16)
            vbuf[slot, blk(c), :] = kv[:, D:].astype(BF16)
            return kv[0:8, 0:LANE]

        qs = {NA - 1: qa[...], NA - 2: proj_q(wcur, blk(NA - 2)).astype(BF16)}
        nxt = NA - 3
        dep = None
        for step, i in enumerate(reversed(range(NA))):
            s = _dot_nt(qs[i], kbuf[slot, 0:(i + 1) * TA, :])
            fill = []
            for t in ([nxt, nxt - 1] if step == 0 else [nxt]):
                if t >= 0:
                    qn = proj_q(wcur, blk(t))
                    qs[t] = qn.astype(BF16)
                    fill.append(qn[0:8])
                elif t == -1:
                    qn = proj_q(wnext, blk(NA - 1))
                    qa[...] = qn.astype(BF16)
                    fill.append(qn[0:8])
                nxt -= 1
            if step >= 1:
                fill.append(pkv(i + 1))
            o, on = softmax_pv(h, slot, i, s, dep)
            pin = side_work(step, [fill[-1], fill[0], o[0:8]])
            if pin is not None:
                n = pin.shape[0]
                on = jnp.concatenate([jnp.maximum(pin, on[:n]), on[n:]], axis=0)
            dep = never(on)
        pkv(0)

    def head_last(h, side_work):
        slot = h % AH
        wcur, wnext = wslot_of(h), wslot_of(h + 1)
        qs = {NA - 1: qa[...], 0: proj_q(wcur, blk(0)).astype(BF16)}
        deps = [None, None]
        for g in range(NA // 2):
            pair = (NA - 1 - g, g)
            ss = [_dot_nt(qs[i], kbuf[slot, 0:(i + 1) * TA, :]) for i in pair]
            qn = None
            if g + 1 < NA // 2:
                for t in (NA - 2 - g, g + 1):
                    qn = proj_q(wcur, blk(t))
                    qs[t] = qn.astype(BF16)
            for k, i in enumerate(pair):
                _, on = softmax_pv(h, slot, i, ss[k], deps[k])
                deps[k] = never(on)
            if qn is not None:
                side_work(g, qn[0:8])
        qa[...] = proj_q(wnext, blk(NA - 1)).astype(BF16)

    for cp in small_copies():
        cp.start()
    w_copy(0, 0).start()
    for cp in small_copies():
        cp.wait()
    for r in range(NCC):
        c_copy(r).start()
    dall = dvec_ref[...].astype(F32)
    for i in range(NT_):
        dtile[i] = jnp.broadcast_to(dall[i:i + 1, :], (8, LANE))
    for c in range(NB):
        zref[c] = 0
    kpad[0:8, :] = jnp.zeros((8, LANE), F32)

    def wkv0_body(r, carry):
        r0 = pl.multiple_of(r * TA, TA)
        convert(0, r0, TA)
        for t in range(AH + 1):
            extract(t, wslot_of(t), r0, TA)
        return carry

    def wq0_body(r, carry):
        r0 = pl.multiple_of(r * TA, TA)
        convert(0, r0, TA)
        extract(0, wslot_of(0), r0, TA)
        return carry

    def proj0(t, w0, buf):
        rows = pl.ds(pl.multiple_of(t * PR, PR), PR)
        w = jnp.concatenate([x_t[wslot_of(e), w0:w0 + DC, :] for e in range(AH)], axis=1)
        y = _dot(c_v[rows, :], w)
        for e in range(AH):
            buf[e, rows, :] = y[:, e * D:(e + 1) * D].astype(BF16)

    def k0_body(t, carry):
        @pl.when(t == XT0)
        def _():
            for i in range(NT_):
                x_copy(i).start()
            w_copy(1, 0).start()

        c_copy(t).wait()
        proj0(t, 0, kbuf)
        return carry

    def v0_body(t, carry):
        proj0(t, DC, vbuf)
        return carry

    nq = QR // TA
    w_copy(0, 0).wait()
    jax.lax.fori_loop(0, nq, wkv0_body, 0)
    w_copy(0, 1).start()
    w_copy(0, 2).start()
    w_copy(0, 3).start()
    jax.lax.fori_loop(0, NCC, k0_body, 0)
    w_copy(0, 1).wait()
    jax.lax.fori_loop(nq, 2 * nq, wkv0_body, 0)
    jax.lax.fori_loop(0, NCC, v0_body, 0)
    w_copy(0, 2).wait()
    w_copy(0, 3).wait()
    jax.lax.fori_loop(2 * nq, 4 * nq, wq0_body, 0)
    for i in range(NT_):
        x_copy(i).wait()
    for r in range(1, NQT):
        w_copy(1, r).start()
    qa[...] = proj_q(wslot_of(0), blk(NA - 1)).astype(BF16)

    nh = NA // 2
    ER = WR // GH
    GR = -(-S // (8 * (H - AH)))
    order = [(0, c) for c in range(nh - 2)] + [(1, c) for c in range(nh - 2)] + [
        (0, nh - 2), (0, nh - 1), (1, nh - 2), (1, nh - 1)]

    def full_body(h, carry):
        for r in range(NQT):
            @pl.when(jnp.logical_and(h < (NG - 1) * GH, h % GH == 2 * r))
            def _():
                w_copy(h // GH + 1, r).wait()

        for t in range(NT_):
            @pl.when(h == 2 * t + 2)
            def _():
                w_copy(t // NQT + 2, t % NQT).start()
                for cp in tile_copies(t):
                    cp.start()

        gslot = jnp.minimum(h // GH + 1, NG - 1) % 2
        e0 = pl.multiple_of((h % GH) * ER, ER)
        hkv = jnp.minimum(h + AH + 1, H - 1)

        def side(step, pins):
            n = ER // CVS // 2
            if step < CVS:
                convert(gslot, e0 + step * 2 * n, n, pins[1])
            for ch in ([2 * step, 2 * step + 1] if step < ND else [step + ND] if step + ND < NA else []):
                isq, c = order[ch]
                if isq:
                    extract(h + 1, wslot_of(h + 1), 2 * DC + c * TA, TA, pins[0])
                else:
                    extract(hkv, wslot_of(h + AH + 1), c * TA, TA, pins[0])
            if step < CVS:
                convert(gslot, e0 + (step * 2 + 1) * n, n, pins[2])
            if CG0 <= step < CG0 + GR:
                return gate_rows(pl.multiple_of(jnp.minimum(h * (8 * GR) + (step - CG0) * 8, S - 8), 8), 8)
            return None

        head_full(h, side)
        return carry

    def last_body(h, carry):
        hq = jnp.minimum(h + 1, H - 1)

        def side(g, pin):
            for c in ([0, 1] if g == 0 else [g + 1]):
                extract(hq, wslot_of(h + 1), 2 * DC + c * TA, TA, pin)

        head_last(h, side)
        return carry

    if not NOHEAD:
        jax.lax.fori_loop(0, H - AH, full_body, 0)
        jax.lax.fori_loop(H - AH, H, last_body, 0)

    sgn_row = jax.lax.broadcasted_iota(jnp.int32, (8, LANE), 0)
    sgn = jnp.where((sgn_row & 1) == 0, 1.0, -1.0).astype(F32)

    for i in range(NT_):
        for cp in tile_copies(i):
            cp.wait()

    RB = 2 * CB
    NR = S // RB
    hp = H // NP
    npin = 32 // NP
    rg = RB // npin

    def tile_body(i, carry):
        sh = shift_ref[i].astype(F32)
        dv = dtile[i, 0:1, :]
        hprev = [None]
        hist = []

        def fwd(b):
            hf = _dot_nt(f_ref[...], ssm_v[i, :, b * CB:(b + 1) * CB])
            kpad[8 + b * CB:8 + (b + 1) * CB, :] = k_t[i, b * CB:(b + 1) * CB, :].astype(F32)
            ks = None
            for t in range(KS):
                term = kpad[8 + b * CB - t:8 + (b + 1) * CB - t, :] * sh[t:t + 1, :]
                ks = term if ks is None else ks + term
            u = (ks * v_t[i, b * CB:(b + 1) * CB, :].astype(F32)).astype(BF16)
            u_v[b * CB:(b + 1) * CB, :] = u
            ufb = _dot(f_ref[...], u)
            w = wf[b // 2]
            for sl in range(CB // 8):
                re = slice(16 * sl, 16 * sl + 8)
                im = slice(16 * sl + 8, 16 * sl + 16)
                w[b % 2, 32 * sl:32 * sl + 16, :] = ufb[16 * sl:16 * sl + 16]
                if hprev[0] is None:
                    w[b % 2, 32 * sl + 16:32 * sl + 32, :] = hf[16 * sl:16 * sl + 16]
                else:
                    w[b % 2, 32 * sl + 16:32 * sl + 24, :] = hf[re] - sgn * hprev[0][im]
                    w[b % 2, 32 * sl + 24:32 * sl + 32, :] = hf[im] + sgn * hprev[0][re]
            hprev[0] = hf
            if HEXT & 1:
                hist.extend([hf[0:8], ufb[0:8]])

        def mac(cblk, sl, pin):
            z = zref[cblk]
            yr = None
            yi = None
            for b in range(cblk + 1):
                wu, wg = wf[b // 2], wf[(cblk - b) // 2]
                a_r = wu[z + b % 2, pl.ds(32 * sl, 8), :]
                a_i = wu[z + b % 2, pl.ds(32 * sl + 8, 8), :]
                g_r = wg[z + (cblk - b) % 2, pl.ds(32 * sl + 16, 8), :]
                g_i = wg[z + (cblk - b) % 2, pl.ds(32 * sl + 24, 8), :]
                tr = a_r * g_r - a_i * g_i
                ti = a_r * g_i + a_i * g_r
                yr = tr if yr is None else yr + tr
                yi = ti if yi is None else yi + ti
            if pin is not None:
                yr = jnp.where(never(pin), 0.0, yr)
            y0 = (cblk % 8) * 2 * CB + 16 * sl
            ctx[z + H, y0:y0 + 16, :] = jnp.concatenate([yr, yi], axis=0).astype(BF16)

        def inv(r):
            y = jnp.concatenate(
                [_dot(finv_ref[...], ctx[H, (c % 8) * 2 * CB:(c % 8 + 1) * 2 * CB, :]) for c in (2 * r, 2 * r + 1)],
                axis=0)
            if HEXT & 2:
                hist.extend([y[0:8], y[CB:CB + 8]])
            rows = slice(r * RB, (r + 1) * RB)
            y = y + u_v[rows, :].astype(F32) * dv
            bpart[r % 2] = (1.0 - gate[rows, :]) * (x_t[i, rows, :].astype(F32) * y)

        for b in range(4):
            fwd(b)
        for r in range(NR):
            cones = [(2 * (r + 1) + k % 2, k // 2) for k in range(32)] if r + 1 < NR else []
            if r == 0:
                cones = [(k % 2, k // 2) for k in range(32)] + cones
            first = npin if r == 0 else 0
            npts = NP * npin - first
            a = None
            for kp in range(NP):
                parts = []
                for t in range(npin):
                    pt = kp * npin + t - first
                    if pt >= 0:
                        for cn in cones[pt * len(cones) // npts:(pt + 1) * len(cones) // npts]:
                            hi = len(hist) + t - PLAG
                            mac(*cn, hist[hi] if hi >= 0 else None)
                    rows = slice(r * RB + t * rg, r * RB + (t + 1) * rg)
                    parts.append(jnp.concatenate([ctx[h, rows, :] for h in range(kp * hp, (kp + 1) * hp)], axis=1))
                ap = _dot(jnp.concatenate(parts, axis=0), wo_t[i, kp * hp * D:(kp + 1) * hp * D, :])
                a = ap if a is None else ap + a
                hist.extend([a[t * rg:t * rg + 8] for t in range(npin)])
                if (kp == INVP and r > 0) or (kp == NP - 2 and r == 0):
                    inv(r)
                for e, fp in enumerate((FP0, FP1)):
                    if kp == fp and 2 * r + 4 + e < NB:
                        fwd(2 * r + 4 + e)
            rows = slice(r * RB, (r + 1) * RB)
            out_t[i, rows, :] = (gate[rows, :] * a + bpart[r % 2]).astype(BF16)
            if (r + 1) * RB == S - OL:
                out_copy(i, 0).start()
        out_copy(i, 1).start()
        return carry

    if not NOTAIL:
        jax.lax.fori_loop(0, NT_, tile_body, 0)
    for i in range(NT_):
        out_copy(i, 0).wait()
        out_copy(i, 1).wait()


@jax.jit
def pallas_gated_mix__compressed_kv_cla__ssm_conv_h3__prompt_kernel(
    A_x: jax.Array,
    A_c_kv: jax.Array,
    A_w_q: jax.Array,
    A_w_uk: jax.Array,
    A_w_uv: jax.Array,
    A_w_o: jax.Array,
    B_q: jax.Array,
    B_k: jax.Array,
    B_v: jax.Array,
    B_shift_k: jax.Array,
    B_ssm_k: jax.Array,
    B_ssm_D: jax.Array,
    gate_w: jax.Array,
):
    del B_q
    fwd, finv = _dft_mats()
    x = A_x.reshape(S, M)
    c = A_c_kv.reshape(S, DC)
    wo = A_w_o.reshape(H * D, M)
    kk = B_k.reshape(S, M)
    vv = B_v.reshape(S, M)
    shift = B_shift_k.reshape(NT_, LANE, KS).transpose(0, 2, 1)
    dvec = B_ssm_D.reshape(NT_, LANE)
    gw = gate_w.reshape(NT_, LANE)

    any_spec = pl.BlockSpec(memory_space=pl.ANY)
    out = pl.pallas_call(
        _kernel,
        out_shape=jax.ShapeDtypeStruct((S, M), BF16),
        in_specs=[any_spec] * 14,
        out_specs=any_spec,
        scratch_shapes=[
            pltpu.VMEM((NT_ + NW, S, LANE), BF16),
            pltpu.VMEM((S, DC), BF16),
            pltpu.VMEM((WR, GH, D), BF16),
            pltpu.VMEM((2, WR * GH, D), F32),
            pltpu.VMEM((TA, D), BF16),
            pltpu.VMEM((AH, S, D), BF16),
            pltpu.VMEM((AH, S, D), BF16),
            pltpu.VMEM((H + 1, S, D), BF16),
            pltpu.VMEM((NT_, H * D, LANE), BF16),
            pltpu.VMEM((NT_, S, LANE), BF16),
            pltpu.VMEM((NT_, S, LANE), BF16),
            pltpu.VMEM((NT_, LANE, S), BF16),
            pltpu.VMEM((S, LANE), F32),
            pltpu.VMEM((S + 32, LANE), F32),
            pltpu.VMEM((NT_, S, LANE), BF16),
            pltpu.VMEM((S, LANE), BF16),
            pltpu.VMEM((2, 2 * CB, LANE), F32),
        ] + [pltpu.VMEM((2, 4 * CB, LANE), F32)] * (NB // 2) + [
            pltpu.VMEM((2 * CB, CB), BF16),
            pltpu.VMEM((CB, 2 * CB), BF16),
            pltpu.VMEM((NT_, 8, LANE), F32),
            pltpu.VMEM((NT_, KS, LANE), BF16),
            pltpu.VMEM((NT_, LANE), BF16),
            pltpu.VMEM((NT_, LANE), BF16),
            pltpu.SMEM((NB,), jnp.int32),
            pltpu.SemaphoreType.DMA((1,)),
            pltpu.SemaphoreType.DMA((NCC,)),
            pltpu.SemaphoreType.DMA((NQT,)),
            pltpu.SemaphoreType.DMA((NT_,)),
            pltpu.SemaphoreType.DMA((1,)),
            pltpu.SemaphoreType.DMA((1,)),
        ],
        compiler_params=pltpu.CompilerParams(vmem_limit_bytes=120 * 1024 * 1024,
                                             disable_bounds_checks=bool(NOBC)),
    )(x, c, A_w_q, A_w_uk, A_w_uv, wo, kk, vv, B_ssm_k,
      shift, dvec, gw, jnp.asarray(fwd, BF16), jnp.asarray(finv, BF16))
    return out.reshape(1, S, M)
```

```python
import math

import numpy as np
import jax
import jax.numpy as jnp
import jax.experimental.pallas as pl
import jax.experimental.pallas.tpu as pltpu

NOHEAD = 0
NOTAIL = 0
UN = 2
CVS = 8
CG0 = 1
ND = 0
PLAG = 4
INVP = 1
FP0 = 2
FP1 = 4
RATE = 12.5
CONE0 = 1.0
INVD = 1
FWD_AT = (0, 0, 0, 0, 5, 6, 9, 10, 15, 17, 23, 25, 30, 32, 37, 39)
WIN0 = 8
WIN = (8, 16, 16, 32, 32, 32, 32, 36)
ORD = 1
EP = 13
CV0 = 1
SA = 0
SB = 1
B1 = 0
B2 = 0
B3 = 0
HEXT = 0

S = 2048
M = 1024
H = 32
D = 128
DC = 512
KS = 4
LANE = 128
NT = M // LANE
TA = 128
NA = S // TA
CB = 128
NB = S // CB
WR = 2 * DC + M
GH = 8
NG = H // GH
NQT = 4
QR = WR // NQT
AH = DC // D
NW = 8
PR = 512
NCC = S // PR
OL = 512

F32 = jnp.float32
BF16 = jnp.bfloat16
NT_DIMS = (((1,), (1,)), ((), ()))
QSCALE = (D ** -0.5) * math.log2(math.e)
NEG = -1e9 * math.log2(math.e)


def _dft_mats():
    ke = np.arange(0, CB, 2, dtype=np.float64).reshape(CB // 16, 1, 8)
    k = np.concatenate([ke, CB - 1 - ke], axis=1)
    n = np.arange(CB, dtype=np.float64)
    th = 2.0 * np.pi * (k[..., None] + 0.5) * n / (2 * CB)
    f = np.stack([np.cos(th), -np.sin(th)], axis=2)
    fe = f[:, 0].reshape(CB, CB)
    inv = np.concatenate([fe[:, 0::2].T, fe[:, 1::2].T], axis=0) / float(CB)
    return f.reshape(2 * CB, CB).astype(np.float32), np.ascontiguousarray(inv.astype(np.float32))


def _dot(a, b):
    return jnp.dot(a, b, preferred_element_type=F32)


def _dot_nt(a, b):
    return jax.lax.dot_general(a, b, NT_DIMS, preferred_element_type=F32)


def _never(v):
    return v > jnp.inf


def _blk(i):
    return slice(i * TA, (i + 1) * TA)


def _kernel(x_hbm, c_hbm, wq_hbm, wk_hbm, wv_hbm, wo_hbm, k_hbm, v_hbm, ssm_hbm,
            shift_hbm, dvec_hbm, gw_hbm, f_hbm, finv_hbm,
            out_hbm,
            x_t, cbuf, lw, st, qa, kv,
            ctx, wo_t, k_t, v_t, ssm_v, gate, out_t, u_v, bpart, ytmp,
            wf0, wf1, wf2, wf3, wf4, wf5, wf6, wf7,
            f_ref, finv_ref, dtile, shift_ref, dvec_ref, gw_ref, zref,
            sem_x, sem_c, sem_w, sem_t, sem_out, sem_s, sem_v):

    wf = (wf0, wf1, wf2, wf3, wf4, wf5, wf6, wf7)

    def x_copy(i):
        return pltpu.make_async_copy(x_hbm.at[:, pl.ds(i * LANE, LANE)], x_t.at[i], sem_x.at[0])

    def c_copy(r):
        rows = pl.ds(pl.multiple_of(r * PR, PR), PR)
        return pltpu.make_async_copy(c_hbm.at[rows], cbuf.at[0, rows], sem_c.at[r])

    def w_copy(g, r):
        src, r0 = ((wk_hbm, 0), (wv_hbm, 0), (wq_hbm, 0), (wq_hbm, QR))[r]
        heads = pl.ds(pl.multiple_of(g * GH, GH), GH)
        return pltpu.make_async_copy(src.at[pl.ds(r0, QR), heads, :], lw.at[pl.ds(r * QR, QR)], sem_w.at[r])

    def tile_copies(i):
        cols = pl.ds(i * LANE, LANE)
        return [
            pltpu.make_async_copy(k_hbm.at[:, cols], k_t.at[i], sem_t.at[i]),
            pltpu.make_async_copy(v_hbm.at[:, cols], v_t.at[i], sem_t.at[i]),
            pltpu.make_async_copy(ssm_hbm.at[cols, :], ssm_v.at[i], sem_t.at[i]),
            pltpu.make_async_copy(wo_hbm.at[pl.ds(DC, H * D - DC), cols], wo_t.at[i], sem_t.at[i]),
        ]

    def spill_copies():
        return [pltpu.make_async_copy(ctx.at[e], out_hbm.at[:, pl.ds(e * D, D)], sem_v.at[0])
                for e in range(AH)]

    def virt_copies():
        cps = [pltpu.make_async_copy(wo_hbm.at[pl.ds(0, DC), pl.ds(i * LANE, LANE)],
                                     x_t.at[NT + NW + i // 2, pl.ds((i % 2) * DC, DC)], sem_v.at[1])
               for i in range(NT)]
        cps.append(pltpu.make_async_copy(out_hbm.at[:, pl.ds(0, DC)], cbuf.at[1], sem_v.at[1]))
        return cps

    def out_copy(i, part):
        rows = (pl.ds(0, S - OL), pl.ds(S - OL, OL))[part]
        return pltpu.make_async_copy(out_t.at[i, rows], out_hbm.at[rows, pl.ds(i * LANE, LANE)], sem_out.at[0])

    def small_copies():
        return [pltpu.make_async_copy(src, dst, sem_s.at[0])
                for src, dst in ((shift_hbm, shift_ref), (dvec_hbm, dvec_ref), (gw_hbm, gw_ref),
                                 (f_hbm, f_ref), (finv_hbm, finv_ref))]

    def convert(slot, r0, n, pin=None):
        w = lw[pl.ds(r0, n)].astype(F32)
        if pin is not None:
            w = jnp.where(_never(pin)[None], 0.0, w)
        st[slot, pl.ds(pl.multiple_of(r0 * GH, GH), n * GH), :] = w.reshape(n * GH, D)

    def extract(h, wslot, r0, n, pin=None):
        w = st[(h >> 3) & 1, pl.ds(GH * r0 + (h & (GH - 1)), n, stride=GH), :] if B2 else st[(h // GH) % 2, pl.ds(GH * r0 + h % GH, n, stride=GH), :]
        if pin is not None:
            w = jnp.where(jnp.concatenate([_never(pin)] * (n // 8), axis=0), 0.0, w)
        x_t[wslot, pl.ds(r0, n), :] = w.astype(BF16)

    def wslot_of(h):
        return NT + ((h & (NW - 1)) if B1 else h % NW)

    def proj_q(wslot, rows):
        xr = jnp.concatenate([x_t[i, rows, :] for i in range(NT)], axis=1)
        return _dot(xr, x_t[wslot, 2 * DC:WR, :]) * QSCALE

    def gate_rows(r0, n):
        gw = gw_ref[...].astype(F32)
        z = None
        for i in range(NT):
            t = x_t[i, pl.ds(r0, n), :].astype(F32) * gw[i:i + 1, :]
            z = t if z is None else z + t
        z = jnp.sum(z, axis=-1, keepdims=True)
        g = jnp.broadcast_to(jax.nn.sigmoid(z), (n, LANE))
        gate[pl.ds(r0, n), :] = g
        return g

    nh = NA // 2
    ER = WR // GH
    GR = S // (8 * H)
    order = [(0, c) for c in range(nh - 2)] + [(1, c) for c in range(nh - 2)] + [
        (0, nh - 2), (0, nh - 1), (1, nh - 2), (1, nh - 1)]
    if ORD:
        order = [(1, c) for c in range(nh - 2)] + [(0, c) for c in range(2 + ND + CV0)] + [(1, nh - 2), (1, nh - 1)] + [
            (0, c) for c in range(2 + ND + CV0, nh)]

    def head(h, kb, q_first, dep):
        virt = h + AH >= H
        wcur, wnext = wslot_of(h), wslot_of(h + 1)
        wkv_slot = jnp.where(virt, NT + NW + (h + AH - H), wslot_of(h + AH))
        csel = virt.astype(jnp.int32)
        gslot = jnp.minimum((h >> 3) + 1, NG - 1) & 1 if B2 else jnp.minimum(h // GH + 1, NG - 1) % 2
        e0 = pl.multiple_of(((h & (GH - 1)) if B2 else h % GH) * ER, ER)
        hq = jnp.minimum(h + 1, H - 1)
        hkv = jnp.minimum(h + AH + 1, H - 1)
        row = jax.lax.broadcasted_iota(jnp.int32, (TA, TA), 0)
        col = jax.lax.broadcasted_iota(jnp.int32, (TA, TA), 1)
        tri = col <= row

        def pkv(c):
            w = jnp.concatenate([x_t[wkv_slot, 0:DC, :], x_t[wkv_slot, DC:2 * DC, :]], axis=1)
            y = _dot(cbuf[csel, _blk(c), :], w)
            kv[kb, _blk(c), :] = y[:, :D].astype(BF16)
            kv[kb + 1, _blk(c), :] = y[:, D:].astype(BF16)
            return y[0:8, 0:LANE]

        def side(step, pins):
            n = ER // CVS // 2
            if CV0 <= step < CV0 + CVS:
                convert(gslot, e0 + (step - CV0) * 2 * n, n, pins[1])
            for ch in ([2 * step, 2 * step + 1] if step < ND else [step + ND] if step + ND < NA else []):
                isq, c = order[ch]
                pin = pins[0] if step < EP else pins[3]
                if isq:
                    extract(hq, wnext, 2 * DC + c * TA, TA, pin)
                else:
                    extract(hkv, wslot_of(h + AH + 1), c * TA, TA, pin)
            if CV0 <= step < CV0 + CVS:
                convert(gslot, e0 + ((step - CV0) * 2 + 1) * n, n, pins[2])
            if CG0 <= step < CG0 + GR:
                return gate_rows(pl.multiple_of(h * (8 * GR) + (step - CG0) * 8, 8), 8)
            return None

        qs = {NA - 1: q_first, NA - 2: proj_q(wcur, _blk(NA - 2)).astype(BF16)}
        nxt = NA - 3
        for step, i in enumerate(reversed(range(NA))):
            L = (i + 1) * TA
            s = _dot_nt(qs[i], kv[kb, 0:L, :])
            fill = []
            for t in ([nxt, nxt - 1] if step == 0 else [nxt]):
                if t >= -1:
                    qn = proj_q(wcur, _blk(t)) if t >= 0 else proj_q(wnext, _blk(NA - 1))
                    qs[t] = qn.astype(BF16)
                    fill.append(qn[0:8])
                nxt -= 1
            if step >= 1:
                fill.append(pkv(i + 1))
            sd = jnp.where(tri, s[:, L - TA:], NEG)
            s = jnp.concatenate([s[:, :L - TA], sd], axis=1) if i > 0 else sd
            m = jnp.max(s, axis=-1, keepdims=True)
            mb = jnp.broadcast_to(m, (TA, LANE))
            if dep is not None:
                mb = jnp.where(dep, 0.0, mb)
            p = jnp.exp2(s - jnp.concatenate([mb] * (L // LANE), axis=1))
            l = jnp.sum(p, axis=-1, keepdims=True)
            o = _dot(p.astype(BF16), kv[kb + 1, 0:L, :])
            lb = jnp.broadcast_to(l, (TA, LANE))
            r0 = pl.reciprocal(lb, approx=True)
            on = o * (r0 * (2.0 - lb * r0))
            ctx[h, _blk(i), :] = on.astype(BF16)
            g = side(step, [fill[-1], fill[0], o[0:8], sd[TA - 8:]])
            if g is not None:
                on = jnp.concatenate([jnp.maximum(g, on[:8]), on[8:]], axis=0)
            dep = _never(on)
        pkv(0)
        return qs[-1], dep

    for cp in small_copies():
        cp.start()
    w_copy(0, 0).start()
    for cp in small_copies():
        cp.wait()
    for r in range(NCC):
        c_copy(r).start()
    dall = dvec_ref[...].astype(F32)
    for i in range(NT):
        dtile[i] = jnp.broadcast_to(dall[i:i + 1, :], (8, LANE))
    for c in range(NB):
        zref[c] = 0

    def wkv0_body(r, carry):
        r0 = pl.multiple_of(r * TA, TA)
        convert(0, r0, TA)
        for t in range(AH + 1):
            extract(t, wslot_of(t), r0, TA)
        return carry

    def wq0_body(r, carry):
        r0 = pl.multiple_of(r * TA, TA)
        convert(0, r0, TA)
        extract(0, wslot_of(0), r0, TA)
        return carry

    def proj0(t, which):
        rows = pl.ds(pl.multiple_of(t * PR, PR), PR)
        w = jnp.concatenate([x_t[wslot_of(e), which * DC:(which + 1) * DC, :] for e in range(AH)], axis=1)
        y = _dot(cbuf[0, rows, :], w)
        for e in range(AH):
            kv[2 * e + which, rows, :] = y[:, e * D:(e + 1) * D].astype(BF16)

    def k0_body(t, carry):
        @pl.when(t == 2)
        def _():
            for i in range(NT):
                x_copy(i).start()
            w_copy(1, 0).start()

        c_copy(t).wait()
        proj0(t, 0)
        return carry

    def v0_body(t, carry):
        proj0(t, 1)
        return carry

    nq = QR // TA
    w_copy(0, 0).wait()
    jax.lax.fori_loop(0, nq, wkv0_body, 0)
    for r in range(1, NQT):
        w_copy(0, r).start()
    jax.lax.fori_loop(0, NCC, k0_body, 0)
    w_copy(0, 1).wait()
    jax.lax.fori_loop(nq, 2 * nq, wkv0_body, 0)
    jax.lax.fori_loop(0, NCC, v0_body, 0)
    w_copy(0, 2).wait()
    w_copy(0, 3).wait()
    jax.lax.fori_loop(2 * nq, 4 * nq, wq0_body, 0)
    for i in range(NT):
        x_copy(i).wait()
    for r in range(1, NQT):
        w_copy(1, r).start()
    qa[...] = proj_q(wslot_of(0), _blk(NA - 1)).astype(BF16)

    def head_body(j, carry):
        h0 = j * UN
        @pl.when(j < (NG - 1) * NQT)
        def _():
            r = j & (NQT - 1)
            dst = lw.at[pl.ds(pl.multiple_of(r * QR, QR), QR)]
            pltpu.make_async_copy(dst, dst, sem_w.at[r]).wait()

        @pl.when(h0 == 2 * NT + 6)
        def _():
            for cp in spill_copies():
                cp.wait()

        @pl.when(h0 == H - AH - 2)
        def _():
            for cp in virt_copies():
                cp.wait()

        def starts_a():
            for t in range(NT):
                @pl.when(h0 == 2 * t + 2)
                def _():
                    w_copy(t // NQT + 2, t % NQT).start()
                    for cp in tile_copies(t):
                        cp.start()

        def starts_b():
            @pl.when(h0 == 2 * NT + 2)
            def _():
                for cp in spill_copies():
                    cp.start()

            @pl.when(h0 == 2 * NT + 6)
            def _():
                for cp in virt_copies():
                    cp.start()

        if SA == 0:
            starts_a()
        if SB == 0:
            starts_b()
        kb0 = 2 * ((h0 & (AH - 1)) if B3 else h0 % AH)
        q, dep = qa[...], None
        for e in range(UN):
            q, dep = head(h0 + e, kb0 + 2 * e, q, dep)
            if SA == e + 1:
                starts_a()
            if SB == e + 1:
                starts_b()
        qa[...] = q
        return carry

    if not NOHEAD:
        jax.lax.fori_loop(0, H // UN, head_body, 0)

    for i in range(NT):
        for cp in tile_copies(i):
            cp.wait()

    RB = 2 * CB
    NR = S // RB
    NP = H // AH - 1
    npin = 4
    rg = RB // npin

    fwd_plan, inv_plan, cone_plan = {}, {}, {}
    for b, pc in enumerate(FWD_AT):
        fwd_plan.setdefault(pc, []).append(b)
    pt = WIN0
    for r in range(NR):
        assert pt >= (FWD_AT[2 * r + 1] + 2) * npin, (r, pt)
        for k in range(32):
            cone_plan.setdefault(pt + k * WIN[r] // 32, []).append((2 * r + k % 2, k // 2))
        pt += WIN[r]
        pc = (pt - 1) // npin + INVD
        while pc in fwd_plan or pc - 1 in fwd_plan:
            pc += 1
        assert pc <= (r + 1) * NP - 2, (r, pc)
        inv_plan.setdefault(pc, []).append(r)

    def tile_body(i, carry):
        sh = shift_ref[i].astype(F32)
        dv = dtile[i, 0:1, :]
        hprev = [None]
        held = {}
        hist = []

        def fwd(b):
            hb = ssm_v[i, :, b * CB:(b + 1) * CB]
            hf = jnp.concatenate([_dot_nt(f_ref[e * CB:(e + 1) * CB, :], hb) for e in range(2)], axis=0)
            if b == 0:
                kk = jnp.concatenate([jnp.zeros((16, LANE), F32), k_t[i, 0:CB, :].astype(F32)], axis=0)
            else:
                kk = k_t[i, b * CB - 16:(b + 1) * CB, :].astype(F32)
            ks = None
            for t in range(KS):
                term = kk[16 - t:16 + CB - t, :] * sh[t:t + 1, :]
                ks = term if ks is None else ks + term
            u = (ks * v_t[i, b * CB:(b + 1) * CB, :].astype(F32)).astype(BF16)
            u_v[b * CB:(b + 1) * CB, :] = u
            uf = jnp.concatenate([_dot(f_ref[e * CB:(e + 1) * CB, :], u) for e in range(2)], axis=0)
            w = wf[b // 2]
            for sl in range(CB // 8):
                re = slice(16 * sl, 16 * sl + 8)
                im = slice(16 * sl + 8, 16 * sl + 16)
                w[b % 2, 32 * sl:32 * sl + 16, :] = uf[16 * sl:16 * sl + 16]
                if hprev[0] is None:
                    w[b % 2, 32 * sl + 16:32 * sl + 32, :] = hf[16 * sl:16 * sl + 16]
                elif sl % 2 == 0:
                    w[b % 2, 32 * sl + 16:32 * sl + 24, :] = hf[re] - hprev[0][im]
                    w[b % 2, 32 * sl + 24:32 * sl + 32, :] = hf[im] + hprev[0][re]
                else:
                    w[b % 2, 32 * sl + 16:32 * sl + 24, :] = hf[re] + hprev[0][im]
                    w[b % 2, 32 * sl + 24:32 * sl + 32, :] = hf[im] - hprev[0][re]
            hprev[0] = hf
            if HEXT:
                hist.extend([hf[0:8], uf[0:8]])

        def mac(cblk, sl, pin):
            z = zref[cblk]
            yr = None
            yi = None
            for b in range(cblk + 1):
                wu, wg = wf[b // 2], wf[(cblk - b) // 2]
                a_r = wu[z + b % 2, pl.ds(32 * sl, 8), :]
                a_i = wu[z + b % 2, pl.ds(32 * sl + 8, 8), :]
                g_r = wg[z + (cblk - b) % 2, pl.ds(32 * sl + 16, 8), :]
                g_i = wg[z + (cblk - b) % 2, pl.ds(32 * sl + 24, 8), :]
                tr = a_r * g_r - a_i * g_i
                ti = a_r * g_i + a_i * g_r
                yr = tr if yr is None else yr + tr
                yi = ti if yi is None else yi + ti
            if pin is not None:
                yr = jnp.where(_never(pin), 0.0, yr)
            y0 = (cblk % 8) * 2 * CB + 16 * (sl // 2)
            if sl % 2 == 0:
                ctx[z + H, y0:y0 + 16, :] = jnp.concatenate([yr, yi], axis=0).astype(BF16)
                held[cblk] = (yr, yi)
            else:
                er, ei = held.pop(cblk)
                ctx[z + H, y0:y0 + 16, :] = jnp.concatenate([er + yr, ei - yi], axis=0).astype(BF16)
                ctx[z + H, CB + y0:CB + y0 + 16, :] = jnp.concatenate([er - yr, ei + yi], axis=0).astype(BF16)

        def inv(r):
            hc = CB // 2
            for e in range(2):
                y0 = ((2 * r + e) % 8) * 2 * CB
                for par in range(2):
                    ytmp[pl.ds(e * CB + par, hc, stride=2), :] = _dot(
                        finv_ref[par * hc:(par + 1) * hc, :], ctx[H, y0 + par * CB:y0 + (par + 1) * CB, :])
            rows = slice(r * RB, (r + 1) * RB)
            y = ytmp[...] + u_v[rows, :].astype(F32) * dv
            g = gate[rows, :]
            bpart[rows, :] = g * kv[i, rows, :].astype(F32) + (1.0 - g) * (x_t[i, rows, :].astype(F32) * y)

        for r in range(NR):
            a = None
            for kp in range(NP):
                pc = r * NP + kp
                parts = []
                for t in range(npin):
                    hi = len(hist) + t - PLAG
                    for cn in cone_plan.get(pc * npin + t, ()):
                        mac(*cn, hist[hi] if hi >= 0 else None)
                    rows = slice(r * RB + t * rg, r * RB + (t + 1) * rg)
                    parts.append(jnp.concatenate(
                        [ctx[h, rows, :] for h in range((kp + 1) * AH, (kp + 2) * AH)], axis=1))
                ap = _dot(jnp.concatenate(parts, axis=0), wo_t[i, kp * DC:(kp + 1) * DC, :])
                a = ap if a is None else ap + a
                hist.extend([a[t * rg:t * rg + 8] for t in range(npin)])
                for rr in inv_plan.get(pc, ()):
                    inv(rr)
                for b in fwd_plan.get(pc, ()):
                    fwd(b)
            rows = slice(r * RB, (r + 1) * RB)
            out_t[i, rows, :] = (gate[rows, :] * a + bpart[rows, :]).astype(BF16)
            if (r + 1) * RB == S - OL:
                out_copy(i, 0).start()
        out_copy(i, 1).start()
        return carry

    if not NOTAIL:
        jax.lax.fori_loop(0, NT, tile_body, 0)
        for i in range(NT):
            out_copy(i, 0).wait()
            out_copy(i, 1).wait()


@jax.jit
def pallas_gated_mix__compressed_kv_cla__ssm_conv_h3__prompt_kernel(
    A_x: jax.Array,
    A_c_kv: jax.Array,
    A_w_q: jax.Array,
    A_w_uk: jax.Array,
    A_w_uv: jax.Array,
    A_w_o: jax.Array,
    B_q: jax.Array,
    B_k: jax.Array,
    B_v: jax.Array,
    B_shift_k: jax.Array,
    B_ssm_k: jax.Array,
    B_ssm_D: jax.Array,
    gate_w: jax.Array,
):
    del B_q
    fwd, finv = _dft_mats()
    x = A_x.reshape(S, M)
    c = A_c_kv.reshape(S, DC)
    wo = A_w_o.reshape(H * D, M)
    kk = B_k.reshape(S, M)
    vv = B_v.reshape(S, M)
    shift = B_shift_k.reshape(NT, LANE, KS).transpose(0, 2, 1)
    dvec = B_ssm_D.reshape(NT, LANE)
    gw = gate_w.reshape(NT, LANE)

    any_spec = pl.BlockSpec(memory_space=pl.ANY)
    out = pl.pallas_call(
        _kernel,
        out_shape=jax.ShapeDtypeStruct((S, M), BF16),
        in_specs=[any_spec] * 14,
        out_specs=any_spec,
        scratch_shapes=[
            pltpu.VMEM((NT + NW + AH, S, LANE), BF16),
            pltpu.VMEM((2, S, DC), BF16),
            pltpu.VMEM((WR, GH, D), BF16),
            pltpu.VMEM((2, WR * GH, D), F32),
            pltpu.VMEM((TA, D), BF16),
            pltpu.VMEM((2 * AH, S, D), BF16),
            pltpu.VMEM((H + 1, S, D), BF16),
            pltpu.VMEM((NT, H * D - DC, LANE), BF16),
            pltpu.VMEM((NT, S, LANE), BF16),
            pltpu.VMEM((NT, S, LANE), BF16),
            pltpu.VMEM((NT, LANE, S), BF16),
            pltpu.VMEM((S, LANE), F32),
            pltpu.VMEM((NT, S, LANE), BF16),
            pltpu.VMEM((S, LANE), BF16),
            pltpu.VMEM((S, LANE), F32),
            pltpu.VMEM((2 * CB, LANE), F32),
        ] + [pltpu.VMEM((2, 4 * CB, LANE), F32)] * (NB // 2) + [
            pltpu.VMEM((2 * CB, CB), BF16),
            pltpu.VMEM((CB, CB), BF16),
            pltpu.VMEM((NT, 8, LANE), F32),
            pltpu.VMEM((NT, KS, LANE), BF16),
            pltpu.VMEM((NT, LANE), BF16),
            pltpu.VMEM((NT, LANE), BF16),
            pltpu.SMEM((NB,), jnp.int32),
            pltpu.SemaphoreType.DMA((1,)),
            pltpu.SemaphoreType.DMA((NCC,)),
            pltpu.SemaphoreType.DMA((NQT,)),
            pltpu.SemaphoreType.DMA((NT,)),
            pltpu.SemaphoreType.DMA((1,)),
            pltpu.SemaphoreType.DMA((1,)),
            pltpu.SemaphoreType.DMA((2,)),
        ],
        compiler_params=pltpu.CompilerParams(vmem_limit_bytes=120 * 1024 * 1024),
    )(x, c, A_w_q, A_w_uk, A_w_uv, wo, kk, vv, B_ssm_k,
      shift, dvec, gw, jnp.asarray(fwd, BF16), jnp.asarray(finv, BF16))
    return out.reshape(1, S, M)
```

```python
import math

import numpy as np
import jax
import jax.numpy as jnp
import jax.experimental.pallas as pl
import jax.experimental.pallas.tpu as pltpu

S = 2048
M = 1024
H = 32
D = 128
DC = 512
KS = 4
LANE = 128
NT = M // LANE
TA = 128
NA = S // TA
CB = 128
NB = S // CB
WR = 2 * DC + M
GH = 8
NG = H // GH
NQT = 4
QR = WR // NQT
AH = DC // D
NW = 8
PR = 512
NCC = S // PR
OL = 512

CV0, CVS = 1, 8
CG0 = 1
EP = 13
PLAG = 4
FWD_AT = (0, 0, 0, 0, 5, 6, 9, 10, 15, 17, 23, 25, 30, 32, 37, 39)
WIN0 = 8
WIN = (8, 16, 16, 32, 32, 32, 32, 36)

F32 = jnp.float32
BF16 = jnp.bfloat16
NT_DIMS = (((1,), (1,)), ((), ()))
QSCALE = (D ** -0.5) * math.log2(math.e)
NEG = -1e9 * math.log2(math.e)


def _dft_mats():
    ke = np.arange(0, CB, 2, dtype=np.float64).reshape(CB // 16, 1, 8)
    k = np.concatenate([ke, CB - 1 - ke], axis=1)
    n = np.arange(CB, dtype=np.float64)
    th = 2.0 * np.pi * (k[..., None] + 0.5) * n / (2 * CB)
    f = np.stack([np.cos(th), -np.sin(th)], axis=2)
    fe = f[:, 0].reshape(CB, CB)
    inv = np.concatenate([fe[:, 0::2].T, fe[:, 1::2].T], axis=0) / float(CB)
    return f.reshape(2 * CB, CB).astype(np.float32), np.ascontiguousarray(inv.astype(np.float32))


def _dot(a, b):
    return jnp.dot(a, b, preferred_element_type=F32)


def _dot_nt(a, b):
    return jax.lax.dot_general(a, b, NT_DIMS, preferred_element_type=F32)


def _never(v):
    return v > jnp.inf


def _blk(i):
    return slice(i * TA, (i + 1) * TA)


def _kernel(x_hbm, c_hbm, wq_hbm, wk_hbm, wv_hbm, wo_hbm, k_hbm, v_hbm, ssm_hbm,
            shift_hbm, dvec_hbm, gw_hbm, f_hbm, finv_hbm,
            out_hbm,
            x_t, cbuf, lw, st, qa, kv,
            ctx, wo_t, k_t, v_t, ssm_v, gate, out_t, u_v, bpart, ytmp,
            wf0, wf1, wf2, wf3, wf4, wf5, wf6, wf7,
            f_ref, finv_ref, dtile, shift_ref, dvec_ref, gw_ref, zref,
            sem_x, sem_c, sem_w, sem_t, sem_out, sem_s, sem_v):

    wf = (wf0, wf1, wf2, wf3, wf4, wf5, wf6, wf7)

    def x_copy(i):
        return pltpu.make_async_copy(x_hbm.at[:, pl.ds(i * LANE, LANE)], x_t.at[i], sem_x.at[0])

    def c_copy(r):
        rows = pl.ds(pl.multiple_of(r * PR, PR), PR)
        return pltpu.make_async_copy(c_hbm.at[rows], cbuf.at[0, rows], sem_c.at[r])

    def w_copy(g, r):
        src, r0 = ((wk_hbm, 0), (wv_hbm, 0), (wq_hbm, 0), (wq_hbm, QR))[r]
        heads = pl.ds(pl.multiple_of(g * GH, GH), GH)
        return pltpu.make_async_copy(src.at[pl.ds(r0, QR), heads, :], lw.at[pl.ds(r * QR, QR)], sem_w.at[r])

    def tile_copies(i):
        cols = pl.ds(i * LANE, LANE)
        return [
            pltpu.make_async_copy(k_hbm.at[:, cols], k_t.at[i], sem_t.at[i]),
            pltpu.make_async_copy(v_hbm.at[:, cols], v_t.at[i], sem_t.at[i]),
            pltpu.make_async_copy(ssm_hbm.at[cols, :], ssm_v.at[i], sem_t.at[i]),
            pltpu.make_async_copy(wo_hbm.at[pl.ds(DC, H * D - DC), cols], wo_t.at[i], sem_t.at[i]),
        ]

    def spill_copies():
        return [pltpu.make_async_copy(ctx.at[e], out_hbm.at[:, pl.ds(e * D, D)], sem_v.at[0])
                for e in range(AH)]

    def virt_copies():
        cps = [pltpu.make_async_copy(wo_hbm.at[pl.ds(0, DC), pl.ds(i * LANE, LANE)],
                                     x_t.at[NT + NW + i // 2, pl.ds((i % 2) * DC, DC)], sem_v.at[1])
               for i in range(NT)]
        cps.append(pltpu.make_async_copy(out_hbm.at[:, pl.ds(0, DC)], cbuf.at[1], sem_v.at[1]))
        return cps

    def out_copy(i, part):
        rows = (pl.ds(0, S - OL), pl.ds(S - OL, OL))[part]
        return pltpu.make_async_copy(out_t.at[i, rows], out_hbm.at[rows, pl.ds(i * LANE, LANE)], sem_out.at[0])

    def small_copies():
        return [pltpu.make_async_copy(src, dst, sem_s.at[0])
                for src, dst in ((shift_hbm, shift_ref), (dvec_hbm, dvec_ref), (gw_hbm, gw_ref),
                                 (f_hbm, f_ref), (finv_hbm, finv_ref))]

    def convert(slot, r0, n, pin=None):
        w = lw[pl.ds(r0, n)].astype(F32)
        if pin is not None:
            w = jnp.where(_never(pin)[None], 0.0, w)
        st[slot, pl.ds(pl.multiple_of(r0 * GH, GH), n * GH), :] = w.reshape(n * GH, D)

    def extract(h, wslot, r0, n, pin=None):
        w = st[(h // GH) % 2, pl.ds(GH * r0 + h % GH, n, stride=GH), :]
        if pin is not None:
            w = jnp.where(jnp.concatenate([_never(pin)] * (n // 8), axis=0), 0.0, w)
        x_t[wslot, pl.ds(r0, n), :] = w.astype(BF16)

    def wslot_of(h):
        return NT + h % NW

    def proj_q(wslot, rows):
        xr = jnp.concatenate([x_t[i, rows, :] for i in range(NT)], axis=1)
        return _dot(xr, x_t[wslot, 2 * DC:WR, :]) * QSCALE

    def gate_rows(r0, n):
        gw = gw_ref[...].astype(F32)
        z = None
        for i in range(NT):
            t = x_t[i, pl.ds(r0, n), :].astype(F32) * gw[i:i + 1, :]
            z = t if z is None else z + t
        z = jnp.sum(z, axis=-1, keepdims=True)
        g = jnp.broadcast_to(jax.nn.sigmoid(z), (n, LANE))
        gate[pl.ds(r0, n), :] = g
        return g

    nh = NA // 2
    ER = WR // GH
    GR = S // (8 * H)
    nkv = CV0 + CVS - (nh - 2)
    order = ([(1, c) for c in range(nh - 2)] + [(0, c) for c in range(nkv)]
             + [(1, nh - 2), (1, nh - 1)] + [(0, c) for c in range(nkv, nh)])

    def head(h, kb, q_first, dep):
        virt = h + AH >= H
        wcur, wnext = wslot_of(h), wslot_of(h + 1)
        wkv_slot = jnp.where(virt, NT + NW + (h + AH - H), wslot_of(h + AH))
        csel = virt.astype(jnp.int32)
        gslot = jnp.minimum(h // GH + 1, NG - 1) % 2
        e0 = pl.multiple_of((h % GH) * ER, ER)
        hq = jnp.minimum(h + 1, H - 1)
        hkv = jnp.minimum(h + AH + 1, H - 1)
        row = jax.lax.broadcasted_iota(jnp.int32, (TA, TA), 0)
        col = jax.lax.broadcasted_iota(jnp.int32, (TA, TA), 1)
        tri = col <= row

        def pkv(c):
            w = jnp.concatenate([x_t[wkv_slot, 0:DC, :], x_t[wkv_slot, DC:2 * DC, :]], axis=1)
            y = _dot(cbuf[csel, _blk(c), :], w)
            kv[kb, _blk(c), :] = y[:, :D].astype(BF16)
            kv[kb + 1, _blk(c), :] = y[:, D:].astype(BF16)
            return y[0:8, 0:LANE]

        def side(step, pins):
            n = ER // CVS // 2
            if CV0 <= step < CV0 + CVS:
                convert(gslot, e0 + (step - CV0) * 2 * n, n, pins[1])
            isq, c = order[step]
            pin = pins[0] if step < EP else pins[3]
            if isq:
                extract(hq, wnext, 2 * DC + c * TA, TA, pin)
            else:
                extract(hkv, wslot_of(h + AH + 1), c * TA, TA, pin)
            if CV0 <= step < CV0 + CVS:
                convert(gslot, e0 + ((step - CV0) * 2 + 1) * n, n, pins[2])
            if CG0 <= step < CG0 + GR:
                return gate_rows(pl.multiple_of(h * (8 * GR) + (step - CG0) * 8, 8), 8)
            return None

        qs = {NA - 1: q_first, NA - 2: proj_q(wcur, _blk(NA - 2)).astype(BF16)}
        nxt = NA - 3
        for step, i in enumerate(reversed(range(NA))):
            L = (i + 1) * TA
            s = _dot_nt(qs[i], kv[kb, 0:L, :])
            fill = []
            for t in ([nxt, nxt - 1] if step == 0 else [nxt]):
                if t >= -1:
                    qn = proj_q(wcur, _blk(t)) if t >= 0 else proj_q(wnext, _blk(NA - 1))
                    qs[t] = qn.astype(BF16)
                    fill.append(qn[0:8])
                nxt -= 1
            if step >= 1:
                fill.append(pkv(i + 1))
            sd = jnp.where(tri, s[:, L - TA:], NEG)
            s = jnp.concatenate([s[:, :L - TA], sd], axis=1) if i > 0 else sd
            m = jnp.max(s, axis=-1, keepdims=True)
            mb = jnp.broadcast_to(m, (TA, LANE))
            if dep is not None:
                mb = jnp.where(dep, 0.0, mb)
            p = jnp.exp2(s - jnp.concatenate([mb] * (L // LANE), axis=1))
            l = jnp.sum(p, axis=-1, keepdims=True)
            o = _dot(p.astype(BF16), kv[kb + 1, 0:L, :])
            lb = jnp.broadcast_to(l, (TA, LANE))
            r0 = pl.reciprocal(lb, approx=True)
            on = o * (r0 * (2.0 - lb * r0))
            ctx[h, _blk(i), :] = on.astype(BF16)
            g = side(step, [fill[-1], fill[0], o[0:8], sd[TA - 8:]])
            if g is not None:
                on = jnp.concatenate([jnp.maximum(g, on[:8]), on[8:]], axis=0)
            dep = _never(on)
        pkv(0)
        return qs[-1], dep

    for cp in small_copies():
        cp.start()
    w_copy(0, 0).start()
    for cp in small_copies():
        cp.wait()
    for r in range(NCC):
        c_copy(r).start()
    dall = dvec_ref[...].astype(F32)
    for i in range(NT):
        dtile[i] = jnp.broadcast_to(dall[i:i + 1, :], (8, LANE))
    for c in range(NB):
        zref[c] = 0

    def wkv0_body(r, carry):
        r0 = pl.multiple_of(r * TA, TA)
        convert(0, r0, TA)
        for t in range(AH + 1):
            extract(t, wslot_of(t), r0, TA)
        return carry

    def wq0_body(r, carry):
        r0 = pl.multiple_of(r * TA, TA)
        convert(0, r0, TA)
        extract(0, wslot_of(0), r0, TA)
        return carry

    def proj0(t, which):
        rows = pl.ds(pl.multiple_of(t * PR, PR), PR)
        w = jnp.concatenate([x_t[wslot_of(e), which * DC:(which + 1) * DC, :] for e in range(AH)], axis=1)
        y = _dot(cbuf[0, rows, :], w)
        for e in range(AH):
            kv[2 * e + which, rows, :] = y[:, e * D:(e + 1) * D].astype(BF16)

    def k0_body(t, carry):
        @pl.when(t == 2)
        def _():
            for i in range(NT):
                x_copy(i).start()
            w_copy(1, 0).start()

        c_copy(t).wait()
        proj0(t, 0)
        return carry

    def v0_body(t, carry):
        proj0(t, 1)
        return carry

    nq = QR // TA
    w_copy(0, 0).wait()
    jax.lax.fori_loop(0, nq, wkv0_body, 0)
    for r in range(1, NQT):
        w_copy(0, r).start()
    jax.lax.fori_loop(0, NCC, k0_body, 0)
    w_copy(0, 1).wait()
    jax.lax.fori_loop(nq, 2 * nq, wkv0_body, 0)
    jax.lax.fori_loop(0, NCC, v0_body, 0)
    w_copy(0, 2).wait()
    w_copy(0, 3).wait()
    jax.lax.fori_loop(2 * nq, 4 * nq, wq0_body, 0)
    for i in range(NT):
        x_copy(i).wait()
    for r in range(1, NQT):
        w_copy(1, r).start()
    qa[...] = proj_q(wslot_of(0), _blk(NA - 1)).astype(BF16)

    def head_body(j, carry):
        h0 = j * 2

        @pl.when(j < (NG - 1) * NQT)
        def _():
            r = j & (NQT - 1)
            dst = lw.at[pl.ds(pl.multiple_of(r * QR, QR), QR)]
            pltpu.make_async_copy(dst, dst, sem_w.at[r]).wait()

        @pl.when(h0 == 2 * NT + 6)
        def _():
            for cp in spill_copies():
                cp.wait()

        @pl.when(h0 == H - AH - 2)
        def _():
            for cp in virt_copies():
                cp.wait()

        for t in range(NT):
            @pl.when(h0 == 2 * t + 2)
            def _():
                w_copy(t // NQT + 2, t % NQT).start()
                for cp in tile_copies(t):
                    cp.start()

        kb0 = 2 * (h0 % AH)
        q, dep = head(h0, kb0, qa[...], None)

        @pl.when(h0 == 2 * NT + 2)
        def _():
            for cp in spill_copies():
                cp.start()

        @pl.when(h0 == 2 * NT + 6)
        def _():
            for cp in virt_copies():
                cp.start()

        q, _ = head(h0 + 1, kb0 + 2, q, dep)
        qa[...] = q
        return carry

    jax.lax.fori_loop(0, H // 2, head_body, 0)

    for i in range(NT):
        for cp in tile_copies(i):
            cp.wait()

    RB = 2 * CB
    NR = S // RB
    NP = H // AH - 1
    npin = 4
    rg = RB // npin

    fwd_plan, inv_plan, cone_plan = {}, {}, {}
    for b, pc in enumerate(FWD_AT):
        fwd_plan.setdefault(pc, []).append(b)
    pt = WIN0
    for r in range(NR):
        assert pt >= (FWD_AT[2 * r + 1] + 2) * npin, (r, pt)
        for k in range(32):
            cone_plan.setdefault(pt + k * WIN[r] // 32, []).append((2 * r + k % 2, k // 2))
        pt += WIN[r]
        pc = (pt - 1) // npin + 1
        while pc in fwd_plan or pc - 1 in fwd_plan:
            pc += 1
        assert pc <= (r + 1) * NP - 2, (r, pc)
        inv_plan.setdefault(pc, []).append(r)

    def tile_body(i, carry):
        sh = shift_ref[i].astype(F32)
        dv = dtile[i, 0:1, :]
        hprev = [None]
        held = {}
        hist = []

        def fwd(b):
            hb = ssm_v[i, :, b * CB:(b + 1) * CB]
            hf = jnp.concatenate([_dot_nt(f_ref[e * CB:(e + 1) * CB, :], hb) for e in range(2)], axis=0)
            if b == 0:
                kk = jnp.concatenate([jnp.zeros((16, LANE), F32), k_t[i, 0:CB, :].astype(F32)], axis=0)
            else:
                kk = k_t[i, b * CB - 16:(b + 1) * CB, :].astype(F32)
            ks = None
            for t in range(KS):
                term = kk[16 - t:16 + CB - t, :] * sh[t:t + 1, :]
                ks = term if ks is None else ks + term
            u = (ks * v_t[i, b * CB:(b + 1) * CB, :].astype(F32)).astype(BF16)
            u_v[b * CB:(b + 1) * CB, :] = u
            uf = jnp.concatenate([_dot(f_ref[e * CB:(e + 1) * CB, :], u) for e in range(2)], axis=0)
            w = wf[b // 2]
            for sl in range(CB // 8):
                re = slice(16 * sl, 16 * sl + 8)
                im = slice(16 * sl + 8, 16 * sl + 16)
                w[b % 2, 32 * sl:32 * sl + 16, :] = uf[16 * sl:16 * sl + 16]
                if hprev[0] is None:
                    w[b % 2, 32 * sl + 16:32 * sl + 32, :] = hf[16 * sl:16 * sl + 16]
                elif sl % 2 == 0:
                    w[b % 2, 32 * sl + 16:32 * sl + 24, :] = hf[re] - hprev[0][im]
                    w[b % 2, 32 * sl + 24:32 * sl + 32, :] = hf[im] + hprev[0][re]
                else:
                    w[b % 2, 32 * sl + 16:32 * sl + 24, :] = hf[re] + hprev[0][im]
                    w[b % 2, 32 * sl + 24:32 * sl + 32, :] = hf[im] - hprev[0][re]
            hprev[0] = hf

        def mac(cblk, sl, pin):
            z = zref[cblk]
            yr = None
            yi = None
            for b in range(cblk + 1):
                wu, wg = wf[b // 2], wf[(cblk - b) // 2]
                a_r = wu[z + b % 2, pl.ds(32 * sl, 8), :]
                a_i = wu[z + b % 2, pl.ds(32 * sl + 8, 8), :]
                g_r = wg[z + (cblk - b) % 2, pl.ds(32 * sl + 16, 8), :]
                g_i = wg[z + (cblk - b) % 2, pl.ds(32 * sl + 24, 8), :]
                tr = a_r * g_r - a_i * g_i
                ti = a_r * g_i + a_i * g_r
                yr = tr if yr is None else yr + tr
                yi = ti if yi is None else yi + ti
            if pin is not None:
                yr = jnp.where(_never(pin), 0.0, yr)
            y0 = (cblk % 8) * 2 * CB + 16 * (sl // 2)
            if sl % 2 == 0:
                ctx[z + H, y0:y0 + 16, :] = jnp.concatenate([yr, yi], axis=0).astype(BF16)
                held[cblk] = (yr, yi)
            else:
                er, ei = held.pop(cblk)
                ctx[z + H, y0:y0 + 16, :] = jnp.concatenate([er + yr, ei - yi], axis=0).astype(BF16)
                ctx[z + H, CB + y0:CB + y0 + 16, :] = jnp.concatenate([er - yr, ei + yi], axis=0).astype(BF16)

        def inv(r):
            hc = CB // 2
            for e in range(2):
                y0 = ((2 * r + e) % 8) * 2 * CB
                for par in range(2):
                    ytmp[pl.ds(e * CB + par, hc, stride=2), :] = _dot(
                        finv_ref[par * hc:(par + 1) * hc, :], ctx[H, y0 + par * CB:y0 + (par + 1) * CB, :])
            rows = slice(r * RB, (r + 1) * RB)
            y = ytmp[0:RB, :] + u_v[rows, :].astype(F32) * dv
            g = gate[rows, :]
            bpart[rows, :] = g * kv[i, rows, :].astype(F32) + (1.0 - g) * (x_t[i, rows, :].astype(F32) * y)

        for r in range(NR):
            a = None
            for kp in range(NP):
                pc = r * NP + kp
                parts = []
                for t in range(npin):
                    hi = len(hist) + t - PLAG
                    for cn in cone_plan.get(pc * npin + t, ()):
                        mac(*cn, hist[hi] if hi >= 0 else None)
                    rows = slice(r * RB + t * rg, r * RB + (t + 1) * rg)
                    parts.append(jnp.concatenate(
                        [ctx[h, rows, :] for h in range((kp + 1) * AH, (kp + 2) * AH)], axis=1))
                ap = _dot(jnp.concatenate(parts, axis=0), wo_t[i, kp * DC:(kp + 1) * DC, :])
                a = ap if a is None else ap + a
                hist.extend([a[t * rg:t * rg + 8] for t in range(npin)])
                for rr in inv_plan.get(pc, ()):
                    inv(rr)
                for b in fwd_plan.get(pc, ()):
                    fwd(b)
            rows = slice(r * RB, (r + 1) * RB)
            out_t[i, rows, :] = (gate[rows, :] * a + bpart[rows, :]).astype(BF16)
            if (r + 1) * RB == S - OL:
                out_copy(i, 0).start()
        out_copy(i, 1).start()
        return carry

    jax.lax.fori_loop(0, NT, tile_body, 0)
    for i in range(NT):
        out_copy(i, 0).wait()
        out_copy(i, 1).wait()


@jax.jit
def pallas_gated_mix__compressed_kv_cla__ssm_conv_h3__prompt_kernel(
    A_x: jax.Array,
    A_c_kv: jax.Array,
    A_w_q: jax.Array,
    A_w_uk: jax.Array,
    A_w_uv: jax.Array,
    A_w_o: jax.Array,
    B_q: jax.Array,
    B_k: jax.Array,
    B_v: jax.Array,
    B_shift_k: jax.Array,
    B_ssm_k: jax.Array,
    B_ssm_D: jax.Array,
    gate_w: jax.Array,
):
    del B_q
    fwd, finv = _dft_mats()
    x = A_x.reshape(S, M)
    c = A_c_kv.reshape(S, DC)
    wo = A_w_o.reshape(H * D, M)
    kk = B_k.reshape(S, M)
    vv = B_v.reshape(S, M)
    shift = B_shift_k.reshape(NT, LANE, KS).transpose(0, 2, 1)
    dvec = B_ssm_D.reshape(NT, LANE)
    gw = gate_w.reshape(NT, LANE)

    any_spec = pl.BlockSpec(memory_space=pl.ANY)
    out = pl.pallas_call(
        _kernel,
        out_shape=jax.ShapeDtypeStruct((S, M), BF16),
        in_specs=[any_spec] * 14,
        out_specs=any_spec,
        scratch_shapes=[
            pltpu.VMEM((NT + NW + AH, S, LANE), BF16),
            pltpu.VMEM((2, S, DC), BF16),
            pltpu.VMEM((WR, GH, D), BF16),
            pltpu.VMEM((2, WR * GH + 32, D), F32),
            pltpu.VMEM((TA, D), BF16),
            pltpu.VMEM((2 * AH, S, D), BF16),
            pltpu.VMEM((H + 1, S, D), BF16),
            pltpu.VMEM((NT, H * D - DC, LANE), BF16),
            pltpu.VMEM((NT, S, LANE), BF16),
            pltpu.VMEM((NT, S, LANE), BF16),
            pltpu.VMEM((NT, LANE, S), BF16),
            pltpu.VMEM((S, LANE), F32),
            pltpu.VMEM((NT, S, LANE), BF16),
            pltpu.VMEM((S, LANE), BF16),
            pltpu.VMEM((S, LANE), F32),
            pltpu.VMEM((2 * CB + 32, LANE), F32),
        ] + [pltpu.VMEM((2, 4 * CB, LANE), F32)] * (NB // 2) + [
            pltpu.VMEM((2 * CB, CB), BF16),
            pltpu.VMEM((CB, CB), BF16),
            pltpu.VMEM((NT, 8, LANE), F32),
            pltpu.VMEM((NT, KS, LANE), BF16),
            pltpu.VMEM((NT, LANE), BF16),
            pltpu.VMEM((NT, LANE), BF16),
            pltpu.SMEM((NB,), jnp.int32),
            pltpu.SemaphoreType.DMA((1,)),
            pltpu.SemaphoreType.DMA((NCC,)),
            pltpu.SemaphoreType.DMA((NQT,)),
            pltpu.SemaphoreType.DMA((NT,)),
            pltpu.SemaphoreType.DMA((1,)),
            pltpu.SemaphoreType.DMA((1,)),
            pltpu.SemaphoreType.DMA((2,)),
        ],
        compiler_params=pltpu.CompilerParams(vmem_limit_bytes=120 * 1024 * 1024),
    )(x, c, A_w_q, A_w_uk, A_w_uv, wo, kk, vv, B_ssm_k,
      shift, dvec, gw, jnp.asarray(fwd, BF16), jnp.asarray(finv, BF16))
    return out.reshape(1, S, M)
```
